```python
import os as _os
_os.environ.setdefault("JAX_PLATFORMS", "cpu")
import jax
import jax.numpy as jnp

def _softmax(x, axis=-1):
    return jax.nn.softmax(x, axis=axis)
def _gelu(x):
    return jax.nn.gelu(x, approximate=True)
def _silu(x):
    return jax.nn.silu(x)
def _sigmoid(x):
    return jax.nn.sigmoid(x)
def _layernorm(x, axis=-1, eps=1e-5):
    m = jnp.mean(x, axis=axis, keepdims=True)
    v = jnp.var(x, axis=axis, keepdims=True)
    return (x - m) / jnp.sqrt(v + eps)
def _scatter_add(tgt, idx, src, axis=0):
    return tgt.at[idx].add(src)
def _segment_sum(src, seg, n):
    return jax.ops.segment_sum(src, seg, n)
class _Rng:
    def __init__(self, key):
        self._k = key
    def _next(self):
        self._k, sub = jax.random.split(self._k)
        return sub
    def normal(self, shape):
        return jax.random.normal(self._next(), shape, dtype=jnp.bfloat16)
    def randint(self, lo, hi, shape):
        return jax.random.randint(self._next(), shape, lo, hi, dtype=jnp.int32)
    def uniform(self, shape, lo=0.0, hi=1.0):
        return jax.random.uniform(self._next(), shape, jnp.bfloat16, lo, hi)
    def permutation(self, n):
        return jax.random.permutation(self._next(), n)


kernel_name = 'gated_mix__softmax_full_mha__spectral_gfnet__prompt'

def setup_inputs():
    _rng = _Rng(jax.random.key(int.from_bytes(__import__("os").urandom(4), "little")))
    _w = (lambda a: (lambda t: t.astype(jnp.bfloat16) if jnp.issubdtype(t.dtype, jnp.floating) else t)(jnp.asarray(a)))
    def _A_setup():
        B, S, D = 1, 2048, 448
        return {
            "x": _w((lambda *s: _rng.normal(s) * 0.05)(B, S, D)),
            "wqkv": _w((lambda *s: _rng.normal(s) * 0.4)(D, 3 * D)),
            "wo": _w((lambda *s: _rng.normal(s) * 0.05)(D, D)),
        }
    _A_in = _A_setup()

    def _B_setup():
        B, S, D = 1, 2048, 448
        Df = D // 2 + 1
        return {
            "x": _w((lambda *s: _rng.normal(s) * 0.05)(B, S, D)),
            "w_r": _w((lambda *s: _rng.normal(s) * 1.6)(S, Df) * 0.02),
            "w_i": _w((lambda *s: _rng.normal(s) * 1.6)(S, Df) * 0.02),
        }
    _B_in = _B_setup()

    return {
        "A_x": _A_in["x"],
        "A_wqkv": _A_in["wqkv"],
        "A_wo": _A_in["wo"],
        "B_x": _B_in["x"],
        "B_w_r": _B_in["w_r"],
        "B_w_i": _B_in["w_i"],
        "gate_w": _w((lambda *s: _rng.normal(s) * 0.05)(448) * 16.0),
    }

def reference(A_x, A_wqkv, A_wo, B_x, B_w_r, B_w_i, gate_w):
    def _A_ref(x, wqkv, wo):
        B, S, D = x.shape
        H = 16; Dh = D // H
        qkv = (lambda x, *d: x.transpose(*d))((x @ wqkv).reshape(B, S, 3, H, Dh), 2, 0, 3, 1, 4)
        q, k, v = qkv[0], qkv[1], qkv[2]
        scale = Dh ** -0.5
        scores = jnp.einsum("bhqd,bhkd->bhqk", q, k) * scale
        p = _softmax(scores, axis=-1)
        o = jnp.einsum("bhqk,bhkd->bhqd", p, v)
        return (lambda x, *d: x.transpose(*d))(o, 0, 2, 1, 3).reshape(B, S, D) @ wo

    def _B_ref(x, w_r, w_i):
        B, S, D = x.shape
        X = (lambda x, axes=(-2,-1): jnp.fft.rfft2(x.astype(jnp.float32), axes=axes))(x, axes=(-2, -1))
        W = w_r + 1j * w_i
        X = X * W
        y = (lambda x, s, axes=(-2,-1): jnp.fft.irfft2(x, s=s, axes=axes).astype(jnp.bfloat16))(X, (S, D), axes=(-2, -1))
        return y

    x = A_x
    g = _sigmoid((x * gate_w).sum(-1, keepdims=True))
    a = _A_ref(x, A_wqkv, A_wo)
    b = _B_ref(x, B_w_r, B_w_i)
    return g * a + (1 - g) * b
```

```python
import functools
import numpy as np
import jax
import jax.numpy as jnp
from jax.experimental import pallas as pl
from jax.experimental.pallas import tpu as pltpu

S = 2048
D = 448
DHALF = D // 2
H = 16
DH = 28
HP = 32
DP = H * HP
GW = 4 * DH
DF = D // 2 + 1
TQ = 512
KC = 256
PC = 128
RG = 8
XC = 512
NQ = S // TQ
NCOL = NQ * H
F32 = jnp.float32
BF16 = jnp.bfloat16
QSCALE = float(DH ** -0.5 * np.log2(np.e))
GATE_ROW = 29
SMAX = 40.0
VMAX = 2.0 ** 60
TN = (((0,), (0,)), ((), ()))
NT = (((1,), (1,)), ((), ()))


def _real_rep(m):
    return np.block([[m.real, -m.imag], [m.imag, m.real]])


@functools.lru_cache(maxsize=None)
def _tables():
    n = np.arange(DHALF)
    me = np.arange(0, DF, 2)
    mo = np.arange(1, DF, 2)
    fd = np.zeros((2, DHALF, 256))
    for j, mm in enumerate((me, mo)):
        ang = 2 * np.pi * np.outer(n, mm) / D
        fd[j, :, :len(mm)] = np.cos(ang)
        fd[j, :, 128:128 + len(mm)] = -np.sin(ang)
    b = np.arange(64)
    gc = [np.exp(-2j * np.pi * (np.outer(np.ones(64), b) * c / S + np.outer(b, b) / 64)) for c in range(32)]
    fa = np.stack([_real_rep(g_) for g_ in gc])
    fb = np.transpose(fa, (0, 2, 1)) / S
    fi = np.zeros((2, DHALF, 256))
    for j, mm in enumerate((me, mo)):
        c = np.where((mm == 0) | (mm == DF - 1), 1.0, 2.0)
        ang = 2 * np.pi * np.outer(n, mm) / D
        fi[j, :, :len(mm)] = c[None, :] * np.cos(ang) / D
        fi[j, :, 128:128 + len(mm)] = -c[None, :] * np.sin(ang) / D
    bf = lambda a: np.asarray(a, np.float32).astype(jnp.bfloat16)
    return (bf(fd.reshape(2 * DHALF, 256)), bf(fa.reshape(32 * 128, 128)), bf(fb.reshape(32 * 128, 128)),
            bf(fi.reshape(2 * DHALF, 256)))


def _cmulc(z, num, den):
    re, im = z
    num = num % den
    if num == 0:
        return z
    if 4 * num == den:
        return (im, -re)
    if 2 * num == den:
        return (-re, -im)
    if 4 * num == 3 * den:
        return (-im, re)
    c = float(np.cos(2 * np.pi * num / den))
    s_ = float(-np.sin(2 * np.pi * num / den))
    if (8 * num) % den == 0:
        r = abs(c)
        a = re * r
        b = im * r
        if c > 0 and s_ < 0:
            return (a + b, b - a)
        if c < 0 and s_ < 0:
            return (b - a, -(a + b))
        if c < 0 and s_ > 0:
            return (-(a + b), a - b)
        return (a - b, a + b)
    return (re * c - im * s_, re * s_ + im * c)


def _add(a, b):
    return (a[0] + b[0], a[1] + b[1])


def _sub(a, b):
    return (a[0] - b[0], a[1] - b[1])


def _fft4(x, sign):
    t0, t1 = _add(x[0], x[2]), _sub(x[0], x[2])
    t2, t3 = _add(x[1], x[3]), _sub(x[1], x[3])
    y0, y2 = _add(t0, t2), _sub(t0, t2)
    ym = (t1[0] + t3[1], t1[1] - t3[0])
    yp = (t1[0] - t3[1], t1[1] + t3[0])
    return [y0, ym, y2, yp] if sign > 0 else [y0, yp, y2, ym]


def _fft8(x, sign):
    e = _fft4(x[0::2], sign)
    o = _fft4(x[1::2], sign)
    o = [_cmulc(o[k], sign * k, 8) for k in range(4)]
    return [_add(e[k], o[k]) for k in range(4)] + [_sub(e[k], o[k]) for k in range(4)]


def _kernel(one_ref, xt_hbm, w_hbm, wo_hbm, wr_hbm, wi_hbm, gw_hbm, fd_hbm, fa_hbm, fb_hbm, fi_hbm,
            out_hbm,
            xt_v, w_v, wo_v, wr_v, wi_v, gw_v, fd_v, fa_v, fb_v, fi_v,
            k_s, qt_s, vt_s, ot_s, wot_s, gate_s, wt_s, wvp_s,
            x_s, p_s, u_s, q_s, yb_s, z_s, wu_s,
            s0, p0, p1, o_v, flag_s, xsems, sems, osems):
    NX = S // XC
    xcp = [pltpu.make_async_copy(xt_hbm.at[:, pl.ds(j * XC, XC)], xt_v.at[:, pl.ds(j * XC, XC)], xsems.at[j])
           for j in range(NX)]
    names = ['fd', 'w', 'gw', 'wr', 'wi', 'fa', 'fb', 'wo', 'fi']
    srcs = [fd_hbm, w_hbm, gw_hbm, wr_hbm, wi_hbm, fa_hbm, fb_hbm, wo_hbm, fi_hbm]
    dsts = [fd_v, w_v, gw_v, wr_v, wi_v, fa_v, fb_v, wo_v, fi_v]
    cp = {n: pltpu.make_async_copy(s, d, sems.at[i]) for i, (n, s, d) in enumerate(zip(names, srcs, dsts))}
    cp['fd'].start()
    for c in xcp:
        c.start()
    cp['w'].start()
    cp['gw'].start()
    cp['fd'].wait()

    for j in range(NX):
        xcp[j].wait()
        cs = pl.ds(j * XC, XC)
        x1 = xt_v[:DHALF, cs].astype(F32)
        x2 = xt_v[DHALF:, cs].astype(F32)
        et = (x1 + x2).astype(BF16)
        ot = (x1 - x2).astype(BF16)
        xe = jax.lax.dot_general(et, fd_v[0:DHALF, :], TN, preferred_element_type=F32)
        x_s[0, cs, :] = xe[:, :128]; x_s[2, cs, :] = xe[:, 128:]
        xo = jax.lax.dot_general(ot, fd_v[DHALF:, :], TN, preferred_element_type=F32)
        x_s[1, cs, :] = xo[:, :128]; x_s[3, cs, :] = xo[:, 128:]
        if j == 0:
            for n in ['wr', 'wi', 'fa', 'fb', 'wo', 'fi']:
                cp[n].start()
    cp['w'].wait(); cp['gw'].wait()
    wt_s[...] = w_v[...].T
    wvt = wt_s[2 * D:, :].astype(F32)
    gw = gw_v[...].astype(F32).reshape(1, D)
    pieces = []
    for h in range(H):
        pieces.append(wvt[DH * h:DH * (h + 1)])
        if h == 0:
            pieces += [jnp.zeros((1, D), F32), gw, jnp.zeros((2, D), F32)]
        else:
            pieces.append(jnp.zeros((HP - DH, D), F32))
    wvp_s[...] = jnp.concatenate(pieces, axis=0).astype(BF16)

    nq = [jnp.zeros((1, PC), F32) for _ in range(4)]
    nk = [jnp.zeros((1, PC), F32) for _ in range(4)]
    for j in range(S // PC):
        cs = pl.ds(j * PC, PC)
        qk = jnp.dot(wt_s[0:2 * D, :], xt_v[:, cs], preferred_element_type=F32)
        q = qk[0:D] * QSCALE
        qt_s[:, cs] = q.astype(BF16)
        for g in range(4):
            qg = q[GW * g:GW * (g + 1)]
            nq[g] = jnp.maximum(nq[g], jnp.sum(qg * qg, axis=0, keepdims=True))
            kg = qk[D + GW * g:D + GW * (g + 1)]
            nk[g] = jnp.maximum(nk[g], jnp.sum(kg * kg, axis=0, keepdims=True))
            kg = jnp.concatenate([kg, jnp.zeros((128 - GW, PC), F32)], axis=0)
            k_s[g, cs, :] = kg.astype(BF16).T
    vmax = jnp.zeros((8, PC), F32)
    for j in range(S // PC):
        cs = pl.ds(j * PC, PC)
        vt = jnp.dot(wvp_s[...], xt_v[:, cs], preferred_element_type=F32)
        gate_s[:, cs] = jnp.broadcast_to(vt[GATE_ROW:GATE_ROW + 1, :], (8, PC))
        rows = jax.lax.broadcasted_iota(jnp.int32, (DP, PC), 0)
        vt_s[:, cs] = jnp.where((rows & (HP - 1)) == DH, 1.0, vt).astype(BF16)
        vmax = jnp.maximum(vmax, jnp.max(jnp.abs(vt).reshape(DP // 8, 8, PC), axis=0))
    bound2 = jnp.max(nq[0]) * jnp.max(nk[0])
    for g in range(1, 4):
        bound2 = jnp.maximum(bound2, jnp.max(nq[g]) * jnp.max(nk[g]))
    safe = jnp.logical_and(bound2 * 1.02 <= SMAX * SMAX, jnp.max(vmax) <= VMAX)
    flag_s[0] = jnp.where(safe, 0, 1).astype(jnp.int32)

    def w_task(j, t, tie=None):
        ref = (wr_v, wi_v)[j]
        cs = pl.ds(t * 512, 512)
        u = pltpu.bitcast(ref[0:DHALF, cs], jnp.int32)
        last = jax.lax.shift_right_logical(pltpu.bitcast(ref[DHALF:DF, cs].astype(F32), jnp.int32), 16)
        up = jnp.concatenate([u, last, jnp.zeros((15, 512), jnp.int32)], axis=0)
        wu_s[j, cs, :] = up.T

    def tied(xs, tie):
        if tie is None:
            return xs
        x0 = jnp.where(tie != tie, tie, xs[0][0])
        return [(x0, xs[0][1])] + xs[1:]

    def p1_task(a0, lt, r0, tie=None):
        xs = [(x_s[lt, pl.ds(512 * a1 + 64 * a0 + r0, RG), :], x_s[2 + lt, pl.ds(512 * a1 + 64 * a0 + r0, RG), :])
              for a1 in range(4)]
        xs = tied(xs, tie)
        ys = _fft4(xs, 1)
        for c0 in range(4):
            y = _cmulc(ys[c0], a0 * c0, 32)
            p_s[lt, pl.ds(512 * c0 + 64 * a0 + r0, RG), :] = y[0]
            p_s[2 + lt, pl.ds(512 * c0 + 64 * a0 + r0, RG), :] = y[1]

    def p2_task(c0, lt, r0, tie=None):
        xs = [(p_s[lt, pl.ds(512 * c0 + 64 * a0 + r0, RG), :], p_s[2 + lt, pl.ds(512 * c0 + 64 * a0 + r0, RG), :])
              for a0 in range(8)]
        xs = tied(xs, tie)
        ys = _fft8(xs, 1)
        for c1 in range(8):
            c = c0 + 4 * c1
            yb_s[pl.ds(128 * c + r0, RG), pl.ds(128 * lt, 128)] = ys[c1][0].astype(BF16)
            yb_s[pl.ds(128 * c + 64 + r0, RG), pl.ds(128 * lt, 128)] = ys[c1][1].astype(BF16)

    def smx_task(c, tie=None):
        HI = jnp.int32(-65536)
        xk = jnp.dot(fa_v[c * 128:(c + 1) * 128, :], yb_s[c * 128:(c + 1) * 128, :], preferred_element_type=F32)
        xr, xi = xk[:64], xk[64:]
        ur = wu_s[0, pl.ds(c, 64, stride=32), :]
        ui = wu_s[1, pl.ds(c, 64, stride=32), :]
        wr = jnp.concatenate([pltpu.bitcast(ur << 16, F32), pltpu.bitcast(ur & HI, F32)], axis=1)
        wi = jnp.concatenate([pltpu.bitcast(ui << 16, F32), pltpu.bitcast(ui & HI, F32)], axis=1)
        y = jnp.concatenate([xr * wr - xi * wi, xr * wi + xi * wr], axis=0).astype(BF16)
        u = jnp.dot(fb_v[c * 128:(c + 1) * 128, :], y, preferred_element_type=F32)
        u_s[0, pl.ds(64 * c, 64), :] = u[:64, :128]; u_s[1, pl.ds(64 * c, 64), :] = u[:64, 128:]
        u_s[2, pl.ds(64 * c, 64), :] = u[64:, :128]; u_s[3, pl.ds(64 * c, 64), :] = u[64:, 128:]

    def ip2_task(c0, lt, r0, tie=None):
        xs = [(u_s[lt, pl.ds(64 * (c0 + 4 * c1) + r0, RG), :], u_s[2 + lt, pl.ds(64 * (c0 + 4 * c1) + r0, RG), :])
              for c1 in range(8)]
        xs = tied(xs, tie)
        ys = _fft8(xs, -1)
        for a0 in range(8):
            y = _cmulc(ys[a0], -a0 * c0, 32)
            q_s[lt, pl.ds(512 * c0 + 64 * a0 + r0, RG), :] = y[0]
            q_s[2 + lt, pl.ds(512 * c0 + 64 * a0 + r0, RG), :] = y[1]

    def ip1_task(a0, lt, r0, tie=None):
        xs = [(q_s[lt, pl.ds(512 * c0 + 64 * a0 + r0, RG), :], q_s[2 + lt, pl.ds(512 * c0 + 64 * a0 + r0, RG), :])
              for c0 in range(4)]
        xs = tied(xs, tie)
        ys = _fft4(xs, -1)
        for a1 in range(4):
            z_s[lt, pl.ds(512 * a1 + 64 * a0 + r0, RG), :] = ys[a1][0].astype(BF16)
            z_s[2 + lt, pl.ds(512 * a1 + 64 * a0 + r0, RG), :] = ys[a1][1].astype(BF16)

    def wo_prep(tie=None):
        wof = wo_v[...].astype(F32)
        pieces = []
        for h in range(H):
            pieces += [wof[DH * h:DH * (h + 1)], jnp.zeros((HP - DH, D), F32)]
        wot_s[...] = jnp.concatenate(pieces, axis=0).astype(BF16).T

    P = functools.partial
    rr = range(0, 64, RG)
    t_p1 = [P(p1_task, a0, lt, r0) for lt in range(2) for r0 in rr for a0 in range(8)]
    t_p2 = [P(p2_task, c0, lt, r0) for lt in range(2) for r0 in rr for c0 in range(4)]
    t_w = [P(w_task, j, t) for j in range(2) for t in range(4)]
    t_smx = [P(smx_task, c) for c in range(32)]
    t_ip2 = [P(ip2_task, c0, lt, r0) for lt in range(2) for r0 in rr for c0 in range(4)]
    t_ip1 = [P(ip1_task, a0, lt, r0) for lt in range(2) for r0 in rr for a0 in range(8)]

    def prepA(col):
        h = col % H
        q0 = pl.multiple_of((col // H) * TQ, TQ)
        g = h // 4
        r0 = pl.multiple_of(g * GW, 16)
        sub = h % 4
        r = jax.lax.broadcasted_iota(jnp.int32, (GW, TQ), 0)
        qg = qt_s[pl.ds(r0, GW), pl.ds(q0, TQ)].astype(F32)
        qm = jnp.where((r >= sub * DH) & (r < sub * DH + DH), qg, 0.0).astype(BF16)
        qm = jnp.concatenate([qm, jnp.zeros((128 - GW, TQ), BF16)], axis=0)
        return g, qm

    def AB(colA, pA, colB, pB, tasks=()):
        tasks = list(tasks)
        nch = S // KC
        KH = KC // 2
        if colA is not None:
            g, qm = prepA(colA)
        if colB is not None:
            h0 = pl.multiple_of((colB % H) * HP, HP)
            q0 = pl.multiple_of((colB // H) * TQ, TQ)
            acc = jnp.zeros((HP, TQ), F32)
        for c in range(nch):
            if colA is not None:
                kc = k_s[g, pl.ds(c * KC, KC), :]
                s = jnp.dot(kc, qm, preferred_element_type=F32)
                pA[pl.ds(c * KH, KH), :] = pltpu.bitcast(jnp.exp2(s).astype(BF16), jnp.int32)
            if colB is not None:
                p = pltpu.bitcast(pB[pl.ds(c * KH, KH), :], BF16)
                vtc = vt_s[pl.ds(h0, HP), pl.ds(c * KC, KC)]
                acc = acc + jnp.dot(vtc, p, preferred_element_type=F32)
            mine = tasks[len(tasks) * c // nch:len(tasks) * (c + 1) // nch]
            for j, t in enumerate(mine):
                r = (KC // 8) * j // len(mine) * 8
                t(tie=(s[r:r + 8, 0:128] if colA is not None else None))
        if colB is not None:
            o = acc * (1.0 / acc[DH:DH + 1, :])
            ot_s[pl.ds(h0, HP), pl.ds(q0, TQ)] = o.astype(BF16)

    AB(0, p0, None, None)

    NIT = NCOL // 2

    def full(i, ta=(), tb=()):
        c = 2 * i
        AB(c + 1, p1, c, p0, ta)
        AB(c + 2, p0, c + 1, p1, tb)

    @pl.when(one_ref[0] == 1)
    def _():
        cp['wr'].wait(); cp['wi'].wait()
        full(0, t_p1 + t_w[:4], t_p2 + t_w[4:])

    @pl.when(one_ref[1] == 1)
    def _():
        cp['fa'].wait(); cp['fb'].wait()
        full(1, t_smx, t_ip2)

    @pl.when(one_ref[2] == 1)
    def _():
        cp['wo'].wait(); cp['fi'].wait()
        full(2, t_ip1, [wo_prep])

    UN = 2
    def body(i, carry):
        for u in range(UN):
            full(3 + UN * i + u)
        return carry
    jax.lax.fori_loop(0, (NIT - 4) // UN, body, 0)
    c = 2 * (NIT - 1)
    AB(c + 1, p1, c, p0)
    AB(None, None, c + 1, p1)

    @pl.when(flag_s[0] == 1)
    def _():
        def col_body(col, carry):
            g, qm = prepA(col)
            h0 = pl.multiple_of((col % H) * HP, HP)
            q0 = pl.multiple_of((col // H) * TQ, TQ)

            def pass1(c, m):
                r0 = pl.multiple_of(c * KC, KC)
                s = jnp.dot(k_s[g, pl.ds(r0, KC), :], qm, preferred_element_type=F32)
                s0[pl.ds(r0, KC), :] = s
                return jnp.maximum(m, jnp.max(s, axis=0, keepdims=True))
            m = jax.lax.fori_loop(0, S // KC, pass1, jnp.full((1, TQ), -jnp.inf, F32))

            def pass2(c, acc):
                r0 = pl.multiple_of(c * KC, KC)
                p = jnp.exp2(s0[pl.ds(r0, KC), :] - m).astype(BF16)
                return acc + jnp.dot(vt_s[pl.ds(h0, HP), pl.ds(r0, KC)], p, preferred_element_type=F32)
            acc = jax.lax.fori_loop(0, S // KC, pass2, jnp.zeros((HP, TQ), F32))
            o = acc * (1.0 / acc[DH:DH + 1, :])
            ot_s[pl.ds(h0, HP), pl.ds(q0, TQ)] = o.astype(BF16)
            return carry
        jax.lax.fori_loop(0, NCOL, col_body, 0)

    RC = 512
    outs = []
    for r in range(S // RC):
        cs = slice(r * RC, (r + 1) * RC)
        a = jnp.dot(wot_s[...], ot_s[:, cs], preferred_element_type=F32)
        ze = jnp.concatenate([z_s[0, cs, :], z_s[2, cs, :]], axis=1)
        zo = jnp.concatenate([z_s[1, cs, :], z_s[3, cs, :]], axis=1)
        e = jax.lax.dot_general(fi_v[0:DHALF, :], ze, NT, preferred_element_type=F32)
        o = jax.lax.dot_general(fi_v[DHALF:, :], zo, NT, preferred_element_type=F32)
        b = jnp.concatenate([e + o, e - o], axis=0)
        g_ = jax.nn.sigmoid(gate_s[0:1, cs])
        o_v[:, cs] = (b + g_ * (a - b)).astype(BF16)
        cpo = pltpu.make_async_copy(o_v.at[:, cs], out_hbm.at[:, cs], osems.at[r])
        cpo.start()
        outs.append(cpo)
    for cpo in outs:
        cpo.wait()


@jax.jit
def pallas_gated_mix__softmax_full_mha__spectral_gfnet__prompt_kernel(A_x, A_wqkv, A_wo, B_x, B_w_r, B_w_i, gate_w):
    xt = A_x.reshape(S, D).T
    fd, fa, fb, fi = _tables()
    ins = [xt, A_wqkv, A_wo, B_w_r.T, B_w_i.T, gate_w, fd, fa, fb, fi]
    vm = lambda a: pltpu.VMEM(a.shape, a.dtype)
    scratch = [vm(a) for a in ins] + [
        pltpu.VMEM((4, S, 128), BF16), pltpu.VMEM((D, S), BF16), pltpu.VMEM((DP, S), BF16), pltpu.VMEM((DP, S), BF16),
        pltpu.VMEM((D, DP), BF16), pltpu.VMEM((8, S), F32), pltpu.VMEM((3 * D, D), BF16), pltpu.VMEM((DP, D), BF16),
    ] + [pltpu.VMEM((4, S, 128), F32) for _ in range(4)] + [
        pltpu.VMEM((32 * 128, 256), BF16), pltpu.VMEM((4, S, 128), BF16), pltpu.VMEM((2, S, 128), jnp.int32),
        pltpu.VMEM((S, TQ), F32), pltpu.VMEM((S // 2, TQ), jnp.int32), pltpu.VMEM((S // 2, TQ), jnp.int32),
        pltpu.VMEM((D, S), BF16), pltpu.SMEM((1,), jnp.int32),
        pltpu.SemaphoreType.DMA((S // XC,)), pltpu.SemaphoreType.DMA((9,)), pltpu.SemaphoreType.DMA((4,)),
    ]
    out = pl.pallas_call(
        _kernel,
        out_shape=jax.ShapeDtypeStruct((D, S), BF16),
        in_specs=[pl.BlockSpec(memory_space=pltpu.SMEM)] + [pl.BlockSpec(memory_space=pltpu.HBM)] * len(ins),
        out_specs=pl.BlockSpec(memory_space=pltpu.HBM),
        scratch_shapes=scratch,
        compiler_params=pltpu.CompilerParams(vmem_limit_bytes=110 * 1024 * 1024),
    )(np.ones((4,), np.int32), *ins)
    return out.T.reshape(1, S, D)
```

```python
import functools
import numpy as np
import jax
import jax.numpy as jnp
from jax.experimental import pallas as pl
from jax.experimental.pallas import tpu as pltpu

S = 2048
D = 448
DHALF = D // 2
H = 16
DH = 28
HP = 32
DP = H * HP
GW = 4 * DH
DF = D // 2 + 1
TQ = 512
KC = 256
PC = 128
RG = 8
NK = 144
TS = 2
OFF = 'A0'
XC = 512
NQ = S // TQ
NCOL = NQ * H
F32 = jnp.float32
BF16 = jnp.bfloat16
QSCALE = float(DH ** -0.5 * np.log2(np.e))
GATE_ROW = 29
SMAX = 40.0
VMAX = 2.0 ** 60
TN = (((0,), (0,)), ((), ()))
NT = (((1,), (1,)), ((), ()))


def _real_rep(m):
    return np.block([[m.real, -m.imag], [m.imag, m.real]])


@functools.lru_cache(maxsize=None)
def _tables():
    n = np.arange(DHALF)
    me = np.arange(0, DF, 2)
    mo = np.arange(1, DF, 2)
    fd = np.zeros((2, DHALF, 256))
    for j, mm in enumerate((me, mo)):
        ang = 2 * np.pi * np.outer(n, mm) / D
        fd[j, :, :len(mm)] = np.cos(ang)
        fd[j, :, 128:128 + len(mm)] = -np.sin(ang)
    b = np.arange(64)
    gc = [np.exp(-2j * np.pi * (np.outer(np.ones(64), b) * c / S + np.outer(b, b) / 64)) for c in range(32)]
    fa = np.stack([_real_rep(g_) for g_ in gc])
    fb = np.transpose(fa, (0, 2, 1)) / S
    fi = np.zeros((2, DHALF, 256))
    for j, mm in enumerate((me, mo)):
        c = np.where((mm == 0) | (mm == DF - 1), 1.0, 2.0)
        ang = 2 * np.pi * np.outer(n, mm) / D
        fi[j, :, :len(mm)] = c[None, :] * np.cos(ang) / D
        fi[j, :, 128:128 + len(mm)] = -c[None, :] * np.sin(ang) / D
    bf = lambda a: np.asarray(a, np.float32).astype(jnp.bfloat16)
    return (bf(fd.reshape(2 * DHALF, 256)), bf(fa.reshape(32 * 128, 128)), bf(fb.reshape(32 * 128, 128)),
            bf(fi.reshape(2 * DHALF, 256)))


def _cmulc(z, num, den):
    re, im = z
    num = num % den
    if num == 0:
        return z
    if 4 * num == den:
        return (im, -re)
    if 2 * num == den:
        return (-re, -im)
    if 4 * num == 3 * den:
        return (-im, re)
    c = float(np.cos(2 * np.pi * num / den))
    s_ = float(-np.sin(2 * np.pi * num / den))
    if (8 * num) % den == 0:
        r = abs(c)
        a = re * r
        b = im * r
        if c > 0 and s_ < 0:
            return (a + b, b - a)
        if c < 0 and s_ < 0:
            return (b - a, -(a + b))
        if c < 0 and s_ > 0:
            return (-(a + b), a - b)
        return (a - b, a + b)
    return (re * c - im * s_, re * s_ + im * c)


def _add(a, b):
    return (a[0] + b[0], a[1] + b[1])


def _sub(a, b):
    return (a[0] - b[0], a[1] - b[1])


def _fft4(x, sign):
    t0, t1 = _add(x[0], x[2]), _sub(x[0], x[2])
    t2, t3 = _add(x[1], x[3]), _sub(x[1], x[3])
    y0, y2 = _add(t0, t2), _sub(t0, t2)
    ym = (t1[0] + t3[1], t1[1] - t3[0])
    yp = (t1[0] - t3[1], t1[1] + t3[0])
    return [y0, ym, y2, yp] if sign > 0 else [y0, yp, y2, ym]


def _fft8(x, sign):
    e = _fft4(x[0::2], sign)
    o = _fft4(x[1::2], sign)
    o = [_cmulc(o[k], sign * k, 8) for k in range(4)]
    return [_add(e[k], o[k]) for k in range(4)] + [_sub(e[k], o[k]) for k in range(4)]


def _kernel(one_ref, xt_hbm, w_hbm, wo_hbm, wr_hbm, wi_hbm, gw_hbm, fd_hbm, fa_hbm, fb_hbm, fi_hbm,
            out_hbm,
            xt_v, w_v, wo_v, wr_v, wi_v, gw_v, fd_v, fa_v, fb_v, fi_v,
            k_s, qt_s, vt_s, ot_s, wot_s, gate_s, wt_s, wvp_s,
            x_s, p_s, u_s, q_s, yb_s, z_s, wu_s,
            s0, p0, p1, qb0, qb1, qb2, qb3, o_v, flag_s, xsems, sems, osems):
    NX = S // XC
    xcp = [pltpu.make_async_copy(xt_hbm.at[:, pl.ds(j * XC, XC)], xt_v.at[:, pl.ds(j * XC, XC)], xsems.at[j])
           for j in range(NX)]
    names = ['fd', 'w', 'gw', 'wr', 'wi', 'fa', 'fb', 'wo', 'fi']
    srcs = [fd_hbm, w_hbm, gw_hbm, wr_hbm, wi_hbm, fa_hbm, fb_hbm, wo_hbm, fi_hbm]
    dsts = [fd_v, w_v, gw_v, wr_v, wi_v, fa_v, fb_v, wo_v, fi_v]
    cp = {n: pltpu.make_async_copy(s, d, sems.at[i]) for i, (n, s, d) in enumerate(zip(names, srcs, dsts))}
    xcp[0].start()
    cp['fd'].start()
    for c in xcp[1:]:
        c.start()
    cp['w'].start()
    with jax.named_scope('fdwait'):
        cp['fd'].wait()

    for j in range(NX):
        with jax.named_scope(f'xwait{j}'):
            xcp[j].wait()
        cs = pl.ds(j * XC, XC)
        x1 = xt_v[:DHALF, cs].astype(F32)
        x2 = xt_v[DHALF:, cs].astype(F32)
        et = (x1 + x2).astype(BF16)
        ot = (x1 - x2).astype(BF16)
        xe = jax.lax.dot_general(et, fd_v[0:DHALF, :], TN, preferred_element_type=F32)
        x_s[0, cs, :] = xe[:, :128]; x_s[2, cs, :] = xe[:, 128:]
        xo = jax.lax.dot_general(ot, fd_v[DHALF:, :], TN, preferred_element_type=F32)
        x_s[1, cs, :] = xo[:, :128]; x_s[3, cs, :] = xo[:, 128:]
    cp['gw'].start()
    with jax.named_scope('wwait'):
        cp['w'].wait(); cp['gw'].wait()
    for n in ['wr', 'wi', 'fa', 'fb', 'wo', 'fi']:
        cp[n].start()
    wt_s[...] = w_v[...].T
    wvt = wt_s[2 * D:, :].astype(F32)
    gw = gw_v[...].astype(F32).reshape(1, D)
    pieces = []
    for h in range(H):
        pieces.append(wvt[DH * h:DH * (h + 1)])
        if h == 0:
            pieces += [jnp.zeros((1, D), F32), gw, jnp.zeros((2, D), F32)]
        else:
            pieces.append(jnp.zeros((HP - DH, D), F32))
    wvp_s[...] = jnp.concatenate(pieces, axis=0).astype(BF16)

    nq = [jnp.zeros((1, PC), F32) for _ in range(4)]
    nk = [jnp.zeros((1, PC), F32) for _ in range(4)]
    for j in range(S // PC):
        cs = pl.ds(j * PC, PC)
        qk = jnp.dot(wt_s[0:2 * D, :], xt_v[:, cs], preferred_element_type=F32)
        q = qk[0:D] * QSCALE
        qt_s[:, cs] = q.astype(BF16)
        for g in range(4):
            qg = q[GW * g:GW * (g + 1)]
            nq[g] = jnp.maximum(nq[g], jnp.sum(qg * qg, axis=0, keepdims=True))
            kg = qk[D + GW * g:D + GW * (g + 1)]
            nk[g] = jnp.maximum(nk[g], jnp.sum(kg * kg, axis=0, keepdims=True))
            kg = jnp.concatenate([kg, jnp.zeros((128 - GW, PC), F32)], axis=0)
            k_s[g, pl.ds(j * PC // 2, PC // 2), :] = pltpu.bitcast(kg.astype(BF16).T, jnp.int32)
    vmax = jnp.zeros((8, PC), F32)
    for j in range(S // PC):
        cs = pl.ds(j * PC, PC)
        vt = jnp.dot(wvp_s[...], xt_v[:, cs], preferred_element_type=F32)
        gate_s[:, cs] = jnp.broadcast_to(vt[GATE_ROW:GATE_ROW + 1, :], (8, PC))
        rows = jax.lax.broadcasted_iota(jnp.int32, (DP, PC), 0)
        vt_s[:, cs] = pltpu.bitcast(jnp.where((rows & (HP - 1)) == DH, 1.0, vt).astype(BF16), jnp.int32)
        vmax = jnp.maximum(vmax, jnp.max(jnp.abs(vt).reshape(DP // 8, 8, PC), axis=0))
    bound2 = jnp.max(nq[0]) * jnp.max(nk[0])
    for g in range(1, 4):
        bound2 = jnp.maximum(bound2, jnp.max(nq[g]) * jnp.max(nk[g]))
    safe = jnp.logical_and(bound2 * 1.02 <= SMAX * SMAX, jnp.max(vmax) <= VMAX)
    flag_s[0] = jnp.where(safe, 0, 1).astype(jnp.int32)

    def w_task(j, t, tie=None):
        ref = (wr_v, wi_v)[j]
        cs = pl.ds(t * 512, 512)
        u = pltpu.bitcast(ref[0:DHALF, cs], jnp.int32)
        last = jax.lax.shift_right_logical(pltpu.bitcast(ref[DHALF:DF, cs].astype(F32), jnp.int32), 16)
        up = jnp.concatenate([u, last, jnp.zeros((15, 512), jnp.int32)], axis=0)
        wu_s[j, cs, :] = up.T

    def tied(xs, tie):
        if tie is None:
            return xs
        x0 = jnp.where(tie != tie, tie, xs[0][0])
        return [(x0, xs[0][1])] + xs[1:]

    def p1_task(a0, lt, r0, tie=None):
        xs = [(x_s[lt, pl.ds(512 * a1 + 64 * a0 + r0, RG), :], x_s[2 + lt, pl.ds(512 * a1 + 64 * a0 + r0, RG), :])
              for a1 in range(4)]
        xs = tied(xs, tie)
        ys = _fft4(xs, 1)
        for c0 in range(4):
            y = _cmulc(ys[c0], a0 * c0, 32)
            p_s[lt, pl.ds(512 * c0 + 64 * a0 + r0, RG), :] = y[0]
            p_s[2 + lt, pl.ds(512 * c0 + 64 * a0 + r0, RG), :] = y[1]

    def p2_task(c0, lt, r0, tie=None):
        xs = [(p_s[lt, pl.ds(512 * c0 + 64 * a0 + r0, RG), :], p_s[2 + lt, pl.ds(512 * c0 + 64 * a0 + r0, RG), :])
              for a0 in range(8)]
        xs = tied(xs, tie)
        ys = _fft8(xs, 1)
        for c1 in range(8):
            c = c0 + 4 * c1
            yb_s[pl.ds(128 * c + r0, RG), pl.ds(128 * lt, 128)] = ys[c1][0].astype(BF16)
            yb_s[pl.ds(128 * c + 64 + r0, RG), pl.ds(128 * lt, 128)] = ys[c1][1].astype(BF16)

    def smx_task(c, tie=None):
        HI = jnp.int32(-65536)
        xk = jnp.dot(fa_v[c * 128:(c + 1) * 128, :], yb_s[c * 128:(c + 1) * 128, :], preferred_element_type=F32)
        xr, xi = xk[:64], xk[64:]
        ur = wu_s[0, pl.ds(c, 64, stride=32), :]
        ui = wu_s[1, pl.ds(c, 64, stride=32), :]
        wr = jnp.concatenate([pltpu.bitcast(ur << 16, F32), pltpu.bitcast(ur & HI, F32)], axis=1)
        wi = jnp.concatenate([pltpu.bitcast(ui << 16, F32), pltpu.bitcast(ui & HI, F32)], axis=1)
        y = jnp.concatenate([xr * wr - xi * wi, xr * wi + xi * wr], axis=0).astype(BF16)
        u = jnp.dot(fb_v[c * 128:(c + 1) * 128, :], y, preferred_element_type=F32)
        u_s[0, pl.ds(64 * c, 64), :] = u[:64, :128]; u_s[1, pl.ds(64 * c, 64), :] = u[:64, 128:]
        u_s[2, pl.ds(64 * c, 64), :] = u[64:, :128]; u_s[3, pl.ds(64 * c, 64), :] = u[64:, 128:]

    def ip2_task(c0, lt, r0, tie=None):
        xs = [(u_s[lt, pl.ds(64 * (c0 + 4 * c1) + r0, RG), :], u_s[2 + lt, pl.ds(64 * (c0 + 4 * c1) + r0, RG), :])
              for c1 in range(8)]
        xs = tied(xs, tie)
        ys = _fft8(xs, -1)
        for a0 in range(8):
            y = _cmulc(ys[a0], -a0 * c0, 32)
            q_s[lt, pl.ds(512 * c0 + 64 * a0 + r0, RG), :] = y[0]
            q_s[2 + lt, pl.ds(512 * c0 + 64 * a0 + r0, RG), :] = y[1]

    def ip1_task(a0, lt, r0, tie=None):
        xs = [(q_s[lt, pl.ds(512 * c0 + 64 * a0 + r0, RG), :], q_s[2 + lt, pl.ds(512 * c0 + 64 * a0 + r0, RG), :])
              for c0 in range(4)]
        xs = tied(xs, tie)
        ys = _fft4(xs, -1)
        for a1 in range(4):
            z_s[lt, pl.ds(512 * a1 + 64 * a0 + r0, RG), :] = ys[a1][0].astype(BF16)
            z_s[2 + lt, pl.ds(512 * a1 + 64 * a0 + r0, RG), :] = ys[a1][1].astype(BF16)

    def wo_prep(tie=None):
        wof = wo_v[...].astype(F32)
        pieces = []
        for h in range(H):
            pieces += [wof[DH * h:DH * (h + 1)], jnp.zeros((HP - DH, D), F32)]
        wot_s[...] = jnp.concatenate(pieces, axis=0).astype(BF16).T

    P = functools.partial
    rr = range(0, 64, RG)
    t_p1 = [P(p1_task, a0, lt, r0) for lt in range(2) for r0 in rr for a0 in range(8)]
    t_p2 = [P(p2_task, c0, lt, r0) for lt in range(2) for r0 in rr for c0 in range(4)]
    t_w = [P(w_task, j, t) for j in range(2) for t in range(4)]
    t_smx = [P(smx_task, c) for c in range(32)]
    t_ip2 = [P(ip2_task, c0, lt, r0) for lt in range(2) for r0 in rr for c0 in range(4)]
    t_ip1 = [P(ip1_task, a0, lt, r0) for lt in range(2) for r0 in rr for a0 in range(8)]

    def prepA(col, qb=None, sub=None):
        h = col % H
        q0 = pl.multiple_of((col // H) * TQ, TQ)
        g = h // 4
        r0 = pl.multiple_of(g * GW, 16)
        if sub is None:
            sub = h % 4
        r = jax.lax.broadcasted_iota(jnp.int32, (GW, TQ), 0)
        qg = qt_s[pl.ds(r0, GW), pl.ds(q0, TQ)].astype(F32)
        qm = jnp.where((r >= sub * DH) & (r < sub * DH + DH), qg, 0.0).astype(BF16)
        qm = jnp.concatenate([qm, jnp.zeros((128 - GW, TQ), BF16)], axis=0)
        if qb is not None:
            for d in range(DH):
                qb[8 * d:8 * d + 8, :] = jnp.broadcast_to(qg[DH * sub + d:DH * sub + d + 1, :], (8, TQ))
        return g, sub, qm

    def tie_row(jb, d):
        k = jb * DH + d
        return (k * ((S - NK) // 8)) // (NK // 16 * DH)

    def vpu_block(jb, g, sub, qb, pA, ss):
        KM = S - NK
        kw = k_s[g, pl.ds(KM // 2 + 8 * jb, 8), :]
        acc0 = acc1 = None
        for d in range(DH):
            lane = DH * sub + d
            kbw = jnp.broadcast_to(kw[:, lane:lane + 1], (8, 128))
            r = tie_row(jb, d)
            cc, r = r // (KC // 8), r % (KC // 8)
            tie = ss[cc][8 * r:8 * r + 8, 128 * (d % 4):128 * (d % 4) + 128]
            kbw = jnp.where(tie != tie, pltpu.bitcast(tie, jnp.int32), kbw)
            kb0 = pltpu.bitcast(kbw << 16, F32)
            kb1 = pltpu.bitcast(kbw & jnp.int32(-65536), F32)
            q = qb[8 * d:8 * d + 8, :]
            t0 = jnp.concatenate([kb0] * (TQ // 128), axis=1) * q
            t1 = jnp.concatenate([kb1] * (TQ // 128), axis=1) * q
            acc0 = t0 if acc0 is None else acc0 + t0
            acc1 = t1 if acc1 is None else acc1 + t1
        p0_ = pltpu.bitcast(jnp.exp2(acc0).astype(BF16).astype(F32), jnp.int32)
        p1_ = pltpu.bitcast(jnp.exp2(acc1).astype(BF16).astype(F32), jnp.int32)
        pA[pl.ds(KM // 2 + 8 * jb, 8), :] = jax.lax.shift_right_logical(p0_, 16) | p1_

    def AB(colA, pA, colB, pB, tasks=(), qb=None, sub=None):
        tasks = list(tasks)
        nch = S // KC
        KH = KC // 2
        nk = NK if qb is not None else 0
        KM = S - nk
        nvb = nk // 16
        if colA is not None:
            g, sub, qm = prepA(colA, qb, sub)
        if colB is not None:
            h0 = pl.multiple_of((colB % H) * HP, HP)
            hh = pl.multiple_of((colB % H) * (HP // 2), HP // 2)
            q0 = pl.multiple_of((colB // H) * TQ, TQ)
            acc = jnp.zeros((HP, TQ), F32)
        ss = []
        for c in range(nch):
            if colA is not None and c * KC < KM:
                n = min(KC, KM - c * KC)
                kc = pltpu.bitcast(k_s[g, pl.ds(c * KH, n // 2), :], BF16)
                s = jnp.dot(kc, qm, preferred_element_type=F32)
                pA[pl.ds(c * KH, n // 2), :] = pltpu.bitcast(jnp.exp2(s).astype(BF16), jnp.int32)
                ss.append(s)
                for jb in range(nvb):
                    if tie_row(jb, DH - 1) // (KC // 8) == c:
                        vpu_block(jb, g, sub, qb, pA, ss)
            if colB is not None:
                p = pltpu.bitcast(pB[pl.ds(c * KH, KH), :], BF16)
                vtc = pltpu.bitcast(vt_s[pl.ds(hh, HP // 2), pl.ds(c * KC, KC)], BF16)
                acc = acc + jnp.dot(vtc, p, preferred_element_type=F32)
            mine = tasks[len(tasks) * c // nch:len(tasks) * (c + 1) // nch]
            for j, t in enumerate(mine):
                r = (n // 8) * j // len(mine) * 8 if colA is not None else 0
                t(tie=(s[r:r + 8, 0:128] if colA is not None else None))
        if colB is not None:
            o = acc * (1.0 / acc[DH:DH + 1, :])
            ot_s[pl.ds(h0, HP), pl.ds(q0, TQ)] = o.astype(BF16)

    AB(0, p0, None, None, qb=qb0 if 'A0' in OFF else None)

    NIT = NCOL // 2

    def full(i, ta=(), tb=(), qbs=(None, None), c4=None):
        c = 2 * i
        if c4 is None:
            c4 = c % 4
        AB(c + 1, p1, c, p0, ta, qb=qbs[0], sub=(c4 + 1) % 4)
        AB(c + 2, p0, c + 1, p1, tb, qb=qbs[1], sub=(c4 + 2) % 4)

    @pl.when(one_ref[0] == 1)
    def _():
        cp['wr'].wait(); cp['wi'].wait()
        full(0, t_p1 + t_w[:4], t_p2 + t_w[4:])

    @pl.when(one_ref[1] == 1)
    def _():
        cp['fa'].wait(); cp['fb'].wait()
        full(1, t_smx, t_ip2)

    @pl.when(one_ref[2] == 1)
    def _():
        cp['wo'].wait(); cp['fi'].wait()
        full(2, t_ip1, [wo_prep], qbs=(qb1 if 'a' in OFF else None, qb0 if 'b' in OFF else None))

    UN = 2
    def body(i, carry):
        for u in range(UN):
            full(3 + UN * i + u, qbs=((qb1, qb0), (qb3, qb2))[u % 2] if NK else (None, None), c4=(2 * (3 + u)) % 4)
        return carry
    jax.lax.fori_loop(0, (NIT - 4) // UN, body, 0)
    c = 2 * (NIT - 1)
    AB(c + 1, p1, c, p0, qb=qb1 if NK else None)
    AB(None, None, c + 1, p1)

    @pl.when(flag_s[0] == 1)
    def _():
        def col_body(col, carry):
            g, _, qm = prepA(col)
            h0 = pl.multiple_of((col % H) * HP, HP)
            hh = pl.multiple_of((col % H) * (HP // 2), HP // 2)
            q0 = pl.multiple_of((col // H) * TQ, TQ)

            def pass1(c, m):
                r0 = pl.multiple_of(c * KC, KC)
                kc = pltpu.bitcast(k_s[g, pl.ds(pl.multiple_of(c * (KC // 2), KC // 2), KC // 2), :], BF16)
                s = jnp.dot(kc, qm, preferred_element_type=F32)
                s0[pl.ds(r0, KC), :] = s
                return jnp.maximum(m, jnp.max(s, axis=0, keepdims=True))
            m = jax.lax.fori_loop(0, S // KC, pass1, jnp.full((1, TQ), -jnp.inf, F32))

            def pass2(c, acc):
                r0 = pl.multiple_of(c * KC, KC)
                p = jnp.exp2(s0[pl.ds(r0, KC), :] - m).astype(BF16)
                vtc = pltpu.bitcast(vt_s[pl.ds(hh, HP // 2), pl.ds(r0, KC)], BF16)
                return acc + jnp.dot(vtc, p, preferred_element_type=F32)
            acc = jax.lax.fori_loop(0, S // KC, pass2, jnp.zeros((HP, TQ), F32))
            o = acc * (1.0 / acc[DH:DH + 1, :])
            ot_s[pl.ds(h0, HP), pl.ds(q0, TQ)] = o.astype(BF16)
            return carry
        jax.lax.fori_loop(0, NCOL, col_body, 0)

    RC = 512
    outs = []
    for r in range(S // RC):
        cs = slice(r * RC, (r + 1) * RC)
        a = jnp.dot(wot_s[...], ot_s[:, cs], preferred_element_type=F32)
        ze = jnp.concatenate([z_s[0, cs, :], z_s[2, cs, :]], axis=1)
        zo = jnp.concatenate([z_s[1, cs, :], z_s[3, cs, :]], axis=1)
        e = jax.lax.dot_general(fi_v[0:DHALF, :], ze, NT, preferred_element_type=F32)
        o = jax.lax.dot_general(fi_v[DHALF:, :], zo, NT, preferred_element_type=F32)
        b = jnp.concatenate([e + o, e - o], axis=0)
        g_ = jax.nn.sigmoid(gate_s[0:1, cs])
        o_v[:, cs] = (b + g_ * (a - b)).astype(BF16)
        cpo = pltpu.make_async_copy(o_v.at[:, cs], out_hbm.at[:, cs], osems.at[r])
        cpo.start()
        outs.append(cpo)
    with jax.named_scope('outwait'):
        for cpo in outs:
            cpo.wait()


@jax.jit
def pallas_gated_mix__softmax_full_mha__spectral_gfnet__prompt_kernel(A_x, A_wqkv, A_wo, B_x, B_w_r, B_w_i, gate_w):
    xt = A_x.reshape(S, D).T
    fd, fa, fb, fi = _tables()
    ins = [xt, A_wqkv, A_wo, B_w_r.T, B_w_i.T, gate_w, fd, fa, fb, fi]
    vm = lambda a: pltpu.VMEM(a.shape, a.dtype)
    scratch = [vm(a) for a in ins] + [
        pltpu.VMEM((4, S // 2, 128), jnp.int32), pltpu.VMEM((D, S), BF16), pltpu.VMEM((DP // 2, S), jnp.int32), pltpu.VMEM((DP, S), BF16),
        pltpu.VMEM((D, DP), BF16), pltpu.VMEM((8, S), F32), pltpu.VMEM((3 * D, D), BF16), pltpu.VMEM((DP, D), BF16),
    ] + [pltpu.VMEM((4, S, 128), F32) for _ in range(4)] + [
        pltpu.VMEM((32 * 128, 256), BF16), pltpu.VMEM((4, S, 128), BF16), pltpu.VMEM((2, S, 128), jnp.int32),
        pltpu.VMEM((S, TQ), F32), pltpu.VMEM((S // 2, TQ), jnp.int32), pltpu.VMEM((S // 2, TQ), jnp.int32),
        pltpu.VMEM((8 * DH, TQ), F32), pltpu.VMEM((8 * DH, TQ), F32), pltpu.VMEM((8 * DH, TQ), F32), pltpu.VMEM((8 * DH, TQ), F32),
        pltpu.VMEM((D, S), BF16), pltpu.SMEM((1,), jnp.int32),
        pltpu.SemaphoreType.DMA((S // XC,)), pltpu.SemaphoreType.DMA((9,)), pltpu.SemaphoreType.DMA((4,)),
    ]
    out = pl.pallas_call(
        _kernel,
        out_shape=jax.ShapeDtypeStruct((D, S), BF16),
        in_specs=[pl.BlockSpec(memory_space=pltpu.SMEM)] + [pl.BlockSpec(memory_space=pltpu.HBM)] * len(ins),
        out_specs=pl.BlockSpec(memory_space=pltpu.HBM),
        scratch_shapes=scratch,
        compiler_params=pltpu.CompilerParams(vmem_limit_bytes=110 * 1024 * 1024),
    )(np.ones((4,), np.int32), *ins)
    return out.T.reshape(1, S, D)
```

```python
import functools
import numpy as np
import jax
import jax.numpy as jnp
from jax.experimental import pallas as pl
from jax.experimental.pallas import tpu as pltpu

S = 2048
D = 448
DHALF = D // 2
H = 16
DH = 28
HP = 32
DP = H * HP
GW = 4 * DH
DF = D // 2 + 1
TQ = 512
KC = 512
PC = 128
RG = 8
NK = 144
TS = 2
OFF = 'A0'
WW = 5
WF = 12
SCHED = (5, 10, 12, 22, 27)
XCH = (256, 256, 512, 1024)
OCH = (512, 512, 512, 384, 128)
XC = 512
NQ = S // TQ
NCOL = NQ * H
F32 = jnp.float32
BF16 = jnp.bfloat16
QSCALE = float(DH ** -0.5 * np.log2(np.e))
GATE_ROW = 29
SMAX = 40.0
VMAX = 2.0 ** 60
TN = (((0,), (0,)), ((), ()))
NT = (((1,), (1,)), ((), ()))


def _real_rep(m):
    return np.block([[m.real, -m.imag], [m.imag, m.real]])


@functools.lru_cache(maxsize=None)
def _tables():
    n = np.arange(DHALF)
    me = np.arange(0, DF, 2)
    mo = np.arange(1, DF, 2)
    fd = np.zeros((2, DHALF, 256))
    for j, mm in enumerate((me, mo)):
        ang = 2 * np.pi * np.outer(n, mm) / D
        fd[j, :, :len(mm)] = np.cos(ang)
        fd[j, :, 128:128 + len(mm)] = -np.sin(ang)
    b = np.arange(64)
    gc = [np.exp(-2j * np.pi * (np.outer(np.ones(64), b) * c / S + np.outer(b, b) / 64)) for c in range(32)]
    fa = np.stack([_real_rep(g_) for g_ in gc])
    fb = np.transpose(fa, (0, 2, 1)) / S
    fi = np.zeros((2, DHALF, 256))
    for j, mm in enumerate((me, mo)):
        c = np.where((mm == 0) | (mm == DF - 1), 1.0, 2.0)
        ang = 2 * np.pi * np.outer(n, mm) / D
        fi[j, :, :len(mm)] = c[None, :] * np.cos(ang) / D
        fi[j, :, 128:128 + len(mm)] = -c[None, :] * np.sin(ang) / D
    bf = lambda a: np.asarray(a, np.float32).astype(jnp.bfloat16)
    return (bf(fd.reshape(2 * DHALF, 256)), bf(fa.reshape(32 * 128, 128)), bf(fb.reshape(32 * 128, 128)),
            bf(fi.reshape(2 * DHALF, 256)))


def _cmulc(z, num, den):
    re, im = z
    num = num % den
    if num == 0:
        return z
    if 4 * num == den:
        return (im, -re)
    if 2 * num == den:
        return (-re, -im)
    if 4 * num == 3 * den:
        return (-im, re)
    c = float(np.cos(2 * np.pi * num / den))
    s_ = float(-np.sin(2 * np.pi * num / den))
    if (8 * num) % den == 0:
        r = abs(c)
        a = re * r
        b = im * r
        if c > 0 and s_ < 0:
            return (a + b, b - a)
        if c < 0 and s_ < 0:
            return (b - a, -(a + b))
        if c < 0 and s_ > 0:
            return (-(a + b), a - b)
        return (a - b, a + b)
    return (re * c - im * s_, re * s_ + im * c)


def _add(a, b):
    return (a[0] + b[0], a[1] + b[1])


def _sub(a, b):
    return (a[0] - b[0], a[1] - b[1])


def _fft4(x, sign):
    t0, t1 = _add(x[0], x[2]), _sub(x[0], x[2])
    t2, t3 = _add(x[1], x[3]), _sub(x[1], x[3])
    y0, y2 = _add(t0, t2), _sub(t0, t2)
    ym = (t1[0] + t3[1], t1[1] - t3[0])
    yp = (t1[0] - t3[1], t1[1] + t3[0])
    return [y0, ym, y2, yp] if sign > 0 else [y0, yp, y2, ym]


def _fft8(x, sign):
    e = _fft4(x[0::2], sign)
    o = _fft4(x[1::2], sign)
    o = [_cmulc(o[k], sign * k, 8) for k in range(4)]
    return [_add(e[k], o[k]) for k in range(4)] + [_sub(e[k], o[k]) for k in range(4)]


def _kernel(xt_hbm, w_hbm, wo_hbm, wr_hbm, wi_hbm, gw_hbm, fd_hbm, fa_hbm, fb_hbm, fi_hbm,
            out_hbm,
            xt_v, w_v, wo_v, wr_v, wi_v, gw_v, fd_v, fa_v, fb_v, fi_v,
            k_s, qt_s, vt_s, ot_s, wot_s, gate_s, wt_s, wvp_s,
            x_s, p_s, u_s, q_s, yb_s, z_s, wu_s,
            s0, p0, p1, qb0, qb1, qb2, qb3, o_v, flag_s, xsems, sems, osems):
    NX = len(XCH)
    xoff = [sum(XCH[:j]) for j in range(NX)]
    xcp = [pltpu.make_async_copy(xt_hbm.at[:, pl.ds(xoff[j], XCH[j])], xt_v.at[:, pl.ds(xoff[j], XCH[j])], xsems.at[j])
           for j in range(NX)]
    names = ['fd', 'w', 'gw', 'wr', 'wi', 'fa', 'fb', 'wo', 'fi']
    srcs = [fd_hbm, w_hbm, gw_hbm, wr_hbm, wi_hbm, fa_hbm, fb_hbm, wo_hbm, fi_hbm]
    dsts = [fd_v, w_v, gw_v, wr_v, wi_v, fa_v, fb_v, wo_v, fi_v]
    cp = {n: pltpu.make_async_copy(s, d, sems.at[i]) for i, (n, s, d) in enumerate(zip(names, srcs, dsts))}
    xcp[0].start()
    cp['fd'].start()
    for c in xcp[1:]:
        c.start()
    cp['w'].start()
    with jax.named_scope('fdwait'):
        cp['fd'].wait()

    for j in range(NX):
        with jax.named_scope(f'xwait{j}'):
            xcp[j].wait()
        cs = pl.ds(xoff[j], XCH[j])
        x1 = xt_v[:DHALF, cs].astype(F32)
        x2 = xt_v[DHALF:, cs].astype(F32)
        et = (x1 + x2).astype(BF16)
        ot = (x1 - x2).astype(BF16)
        xe = jax.lax.dot_general(et, fd_v[0:DHALF, :], TN, preferred_element_type=F32)
        x_s[0, cs, :] = xe[:, :128]; x_s[2, cs, :] = xe[:, 128:]
        xo = jax.lax.dot_general(ot, fd_v[DHALF:, :], TN, preferred_element_type=F32)
        x_s[1, cs, :] = xo[:, :128]; x_s[3, cs, :] = xo[:, 128:]
    cp['gw'].start()
    with jax.named_scope('wwait'):
        cp['w'].wait(); cp['gw'].wait()
    for n in ['wr', 'wi', 'fa', 'fb', 'wo', 'fi']:
        cp[n].start()
    wt = w_v[...].T
    gw = gw_v[...].reshape(1, D)
    wt_s[...] = jnp.concatenate([wt[0:2 * D], gw, jnp.zeros((15, D), BF16)], axis=0)
    wvp_s[...] = wt[2 * D:]

    def w_task(j, t, tie=None):
        ref = (wr_v, wi_v)[j]
        cs = pl.ds(t * 512, 512)
        u = pltpu.bitcast(ref[0:DHALF, cs], jnp.int32)
        last = jax.lax.shift_right_logical(pltpu.bitcast(ref[DHALF:DF, cs].astype(F32), jnp.int32), 16)
        up = jnp.concatenate([u, last, jnp.zeros((15, 512), jnp.int32)], axis=0)
        wu_s[j, cs, :] = up.T

    def tied(xs, tie):
        if tie is None:
            return xs
        x0 = jnp.where(tie != tie, tie, xs[0][0])
        return [(x0, xs[0][1])] + xs[1:]

    def p1_task(a0, lt, r0, tie=None):
        xs = [(x_s[lt, pl.ds(512 * a1 + 64 * a0 + r0, RG), :], x_s[2 + lt, pl.ds(512 * a1 + 64 * a0 + r0, RG), :])
              for a1 in range(4)]
        xs = tied(xs, tie)
        ys = _fft4(xs, 1)
        for c0 in range(4):
            y = _cmulc(ys[c0], a0 * c0, 32)
            p_s[lt, pl.ds(512 * c0 + 64 * a0 + r0, RG), :] = y[0]
            p_s[2 + lt, pl.ds(512 * c0 + 64 * a0 + r0, RG), :] = y[1]

    def p2_task(c0, lt, r0, tie=None):
        xs = [(p_s[lt, pl.ds(512 * c0 + 64 * a0 + r0, RG), :], p_s[2 + lt, pl.ds(512 * c0 + 64 * a0 + r0, RG), :])
              for a0 in range(8)]
        xs = tied(xs, tie)
        ys = _fft8(xs, 1)
        for c1 in range(8):
            c = c0 + 4 * c1
            yb_s[pl.ds(128 * c + r0, RG), pl.ds(128 * lt, 128)] = ys[c1][0].astype(BF16)
            yb_s[pl.ds(128 * c + 64 + r0, RG), pl.ds(128 * lt, 128)] = ys[c1][1].astype(BF16)

    def smx_task(c, tie=None):
        HI = jnp.int32(-65536)
        xk = jnp.dot(fa_v[c * 128:(c + 1) * 128, :], yb_s[c * 128:(c + 1) * 128, :], preferred_element_type=F32)
        xr, xi = xk[:64], xk[64:]
        ur = wu_s[0, pl.ds(c, 64, stride=32), :]
        ui = wu_s[1, pl.ds(c, 64, stride=32), :]
        wr = jnp.concatenate([pltpu.bitcast(ur << 16, F32), pltpu.bitcast(ur & HI, F32)], axis=1)
        wi = jnp.concatenate([pltpu.bitcast(ui << 16, F32), pltpu.bitcast(ui & HI, F32)], axis=1)
        y = jnp.concatenate([xr * wr - xi * wi, xr * wi + xi * wr], axis=0).astype(BF16)
        u = jnp.dot(fb_v[c * 128:(c + 1) * 128, :], y, preferred_element_type=F32)
        u_s[0, pl.ds(64 * c, 64), :] = u[:64, :128]; u_s[1, pl.ds(64 * c, 64), :] = u[:64, 128:]
        u_s[2, pl.ds(64 * c, 64), :] = u[64:, :128]; u_s[3, pl.ds(64 * c, 64), :] = u[64:, 128:]

    def ip2_task(c0, lt, r0, tie=None):
        xs = [(u_s[lt, pl.ds(64 * (c0 + 4 * c1) + r0, RG), :], u_s[2 + lt, pl.ds(64 * (c0 + 4 * c1) + r0, RG), :])
              for c1 in range(8)]
        xs = tied(xs, tie)
        ys = _fft8(xs, -1)
        for a0 in range(8):
            y = _cmulc(ys[a0], -a0 * c0, 32)
            q_s[lt, pl.ds(512 * c0 + 64 * a0 + r0, RG), :] = y[0]
            q_s[2 + lt, pl.ds(512 * c0 + 64 * a0 + r0, RG), :] = y[1]

    def ip1_task(a0, lt, r0, tie=None):
        xs = [(q_s[lt, pl.ds(512 * c0 + 64 * a0 + r0, RG), :], q_s[2 + lt, pl.ds(512 * c0 + 64 * a0 + r0, RG), :])
              for c0 in range(4)]
        xs = tied(xs, tie)
        ys = _fft4(xs, -1)
        for a1 in range(4):
            z_s[lt, pl.ds(512 * a1 + 64 * a0 + r0, RG), :] = ys[a1][0].astype(BF16)
            z_s[2 + lt, pl.ds(512 * a1 + 64 * a0 + r0, RG), :] = ys[a1][1].astype(BF16)

    def wo_prep(tie=None):
        wof = wo_v[...].astype(F32)
        pieces = []
        for h in range(H):
            pieces += [wof[DH * h:DH * (h + 1)], jnp.zeros((HP - DH, D), F32)]
        wot_s[...] = jnp.concatenate(pieces, axis=0).astype(BF16).T

    P = functools.partial
    rr = range(0, 64, RG)
    t_p1 = [P(p1_task, a0, lt, r0) for lt in range(2) for r0 in rr for a0 in range(8)]
    t_p2 = [P(p2_task, c0, lt, r0) for lt in range(2) for r0 in rr for c0 in range(4)]
    t_w = [P(w_task, j, t) for j in range(2) for t in range(4)]
    t_smx = [P(smx_task, c) for c in range(32)]
    t_ip2 = [P(ip2_task, c0, lt, r0) for lt in range(2) for r0 in rr for c0 in range(4)]
    t_ip1 = [P(ip1_task, a0, lt, r0) for lt in range(2) for r0 in rr for a0 in range(8)]

    def run_tasks(tasks, res):
        nr = res.shape[0] // 8
        for j, t in enumerate(tasks):
            r = nr * j // len(tasks) * 8
            t(tie=res[r:r + 8, 0:128])

    def share(tasks, a, b, j):
        if not a <= j < b:
            return []
        return tasks[len(tasks) * (j - a) // (b - a):len(tasks) * (j - a + 1) // (b - a)]

    PA, PB, WE, SE, IE = SCHED

    def side(j):
        return (share(t_p1, 0, PA, j) + share(t_p2, PA, PB, j) + share(t_w, WW, WE, j) + share(t_smx, WF, SE, j)
                + share(t_ip2, SE, IE, j) + share(t_ip1, IE, 32, j) + share([wo_prep], 30, 31, j))

    def waits(j):
        if j == WW:
            cp['wr'].wait(); cp['wi'].wait()
        if j == WF:
            cp['fa'].wait(); cp['fb'].wait(); cp['wo'].wait(); cp['fi'].wait()

    nq = [jnp.zeros((1, PC), F32) for _ in range(4)]
    nk = [jnp.zeros((1, PC), F32) for _ in range(4)]
    for j in range(S // PC):
        waits(j)
        cs = pl.ds(j * PC, PC)
        qk = jnp.dot(wt_s[...], xt_v[:, cs], preferred_element_type=F32)
        gate_s[:, cs] = jnp.broadcast_to(qk[2 * D:2 * D + 1, :], (8, PC))
        q = qk[0:D] * QSCALE
        qt_s[:, cs] = q.astype(BF16)
        for g in range(4):
            qg = q[GW * g:GW * (g + 1)]
            nq[g] = jnp.maximum(nq[g], jnp.sum(qg * qg, axis=0, keepdims=True))
            kg = qk[D + GW * g:D + GW * (g + 1)]
            nk[g] = jnp.maximum(nk[g], jnp.sum(kg * kg, axis=0, keepdims=True))
            kg = jnp.concatenate([kg, jnp.zeros((128 - GW, PC), F32)], axis=0)
            k_s[g, pl.ds(j * PC // 2, PC // 2), :] = pltpu.bitcast(kg.astype(BF16).T, jnp.int32)
        run_tasks(side(j), qk)
    vmax = jnp.zeros((8, PC), F32)
    for j in range(S // PC):
        waits(16 + j)
        cs = pl.ds(j * PC, PC)
        vt = jnp.dot(wvp_s[...], xt_v[:, cs], preferred_element_type=F32)
        tail = jnp.concatenate([jnp.ones((1, PC), F32), jnp.zeros((HP - DH - 1, PC), F32)], axis=0)
        pieces = []
        for h in range(H):
            pieces += [vt[DH * h:DH * (h + 1)], tail]
        vt_s[:, cs] = pltpu.bitcast(jnp.concatenate(pieces, axis=0).astype(BF16), jnp.int32)
        vmax = jnp.maximum(vmax, jnp.max(jnp.abs(vt).reshape(D // 8, 8, PC), axis=0))
        run_tasks(side(16 + j), vt)
    bound2 = jnp.max(nq[0]) * jnp.max(nk[0])
    for g in range(1, 4):
        bound2 = jnp.maximum(bound2, jnp.max(nq[g]) * jnp.max(nk[g]))
    safe = jnp.logical_and(bound2 * 1.02 <= SMAX * SMAX, jnp.max(vmax) <= VMAX)
    flag_s[0] = jnp.where(safe, 0, 1).astype(jnp.int32)

    def prepA(col, qb=None, sub=None):
        h = col % H
        q0 = pl.multiple_of((col // H) * TQ, TQ)
        g = h // 4
        r0 = pl.multiple_of(g * GW, 16)
        if sub is None:
            sub = h % 4
        r = jax.lax.broadcasted_iota(jnp.int32, (GW, TQ), 0)
        qg = qt_s[pl.ds(r0, GW), pl.ds(q0, TQ)].astype(F32)
        qm = jnp.where((r >= sub * DH) & (r < sub * DH + DH), qg, 0.0).astype(BF16)
        qm = jnp.concatenate([qm, jnp.zeros((128 - GW, TQ), BF16)], axis=0)
        if qb is not None:
            for d in range(DH):
                qb[8 * d:8 * d + 8, :] = jnp.broadcast_to(qg[DH * sub + d:DH * sub + d + 1, :], (8, TQ))
        return g, sub, qm

    def tie_row(jb, d):
        k = jb * DH + d
        return (k * ((S - NK) // 8)) // (NK // 16 * DH)

    def vpu_block(jb, g, sub, qb, pA, ss):
        KM = S - NK
        kw = k_s[g, pl.ds(KM // 2 + 8 * jb, 8), :]
        acc0 = acc1 = None
        for d in range(DH):
            lane = DH * sub + d
            kbw = jnp.broadcast_to(kw[:, lane:lane + 1], (8, 128))
            r = tie_row(jb, d)
            cc, r = r // (KC // 8), r % (KC // 8)
            tie = ss[cc][8 * r:8 * r + 8, 128 * (d % 4):128 * (d % 4) + 128]
            if d % TS == 0:
                kbw = jnp.where(tie != tie, pltpu.bitcast(tie, jnp.int32), kbw)
            kb0 = pltpu.bitcast(kbw << 16, F32)
            kb1 = pltpu.bitcast(kbw & jnp.int32(-65536), F32)
            q = qb[8 * d:8 * d + 8, :]
            t0 = jnp.concatenate([kb0] * (TQ // 128), axis=1) * q
            t1 = jnp.concatenate([kb1] * (TQ // 128), axis=1) * q
            acc0 = t0 if acc0 is None else acc0 + t0
            acc1 = t1 if acc1 is None else acc1 + t1
        p0_ = pltpu.bitcast(jnp.exp2(acc0).astype(BF16).astype(F32), jnp.int32)
        p1_ = pltpu.bitcast(jnp.exp2(acc1).astype(BF16).astype(F32), jnp.int32)
        pA[pl.ds(KM // 2 + 8 * jb, 8), :] = jax.lax.shift_right_logical(p0_, 16) | p1_

    def AB(colA, pA, colB, pB, tasks=(), qb=None, sub=None):
        tasks = list(tasks)
        nch = S // KC
        KH = KC // 2
        nk = NK if qb is not None else 0
        KM = S - nk
        nvb = nk // 16
        if colA is not None:
            g, sub, qm = prepA(colA, qb, sub)
        if colB is not None:
            h0 = pl.multiple_of((colB % H) * HP, HP)
            hh = pl.multiple_of((colB % H) * (HP // 2), HP // 2)
            q0 = pl.multiple_of((colB // H) * TQ, TQ)
            acc = jnp.zeros((HP, TQ), F32)
        ss = []
        for c in range(nch):
            if colA is not None and c * KC < KM:
                n = min(KC, KM - c * KC)
                kc = pltpu.bitcast(k_s[g, pl.ds(c * KH, n // 2), :], BF16)
                s = jnp.dot(kc, qm, preferred_element_type=F32)
                pA[pl.ds(c * KH, n // 2), :] = pltpu.bitcast(jnp.exp2(s).astype(BF16), jnp.int32)
                ss.append(s)
                for jb in range(nvb):
                    if tie_row(jb, DH - 1) // (KC // 8) == c:
                        vpu_block(jb, g, sub, qb, pA, ss)
            if colB is not None:
                p = pltpu.bitcast(pB[pl.ds(c * KH, KH), :], BF16)
                vtc = pltpu.bitcast(vt_s[pl.ds(hh, HP // 2), pl.ds(c * KC, KC)], BF16)
                acc = acc + jnp.dot(vtc, p, preferred_element_type=F32)
            mine = tasks[len(tasks) * c // nch:len(tasks) * (c + 1) // nch]
            for j, t in enumerate(mine):
                r = (n // 8) * j // len(mine) * 8 if colA is not None else 0
                t(tie=(s[r:r + 8, 0:128] if colA is not None else None))
        if colB is not None:
            o = acc * (1.0 / acc[DH:DH + 1, :])
            ot_s[pl.ds(h0, HP), pl.ds(q0, TQ)] = o.astype(BF16)

    AB(0, p0, None, None, qb=qb0 if 'A0' in OFF else None)

    NIT = NCOL // 2

    def full(i, ta=(), tb=(), qbs=(None, None), c4=None):
        c = 2 * i
        if c4 is None:
            c4 = c % 4
        AB(c + 1, p1, c, p0, ta, qb=qbs[0], sub=(c4 + 1) % 4)
        AB(c + 2, p0, c + 1, p1, tb, qb=qbs[1], sub=(c4 + 2) % 4)

    UN = 2

    def body(i, carry):
        for u in range(UN):
            full(UN * i + u, qbs=((qb1, qb0), (qb3, qb2))[u % 2] if NK else (None, None), c4=(2 * u) % 4)
        return carry
    jax.lax.fori_loop(0, (NIT - 2) // UN, body, 0)
    full(NIT - 2, qbs=(qb1, qb0) if NK else (None, None))
    c = 2 * (NIT - 1)
    AB(c + 1, p1, c, p0, qb=qb1 if NK else None)
    AB(None, None, c + 1, p1)

    @pl.when(flag_s[0] == 1)
    def _():
        def col_body(col, carry):
            g, _, qm = prepA(col)
            h0 = pl.multiple_of((col % H) * HP, HP)
            hh = pl.multiple_of((col % H) * (HP // 2), HP // 2)
            q0 = pl.multiple_of((col // H) * TQ, TQ)

            def pass1(c, m):
                r0 = pl.multiple_of(c * KC, KC)
                kc = pltpu.bitcast(k_s[g, pl.ds(pl.multiple_of(c * (KC // 2), KC // 2), KC // 2), :], BF16)
                s = jnp.dot(kc, qm, preferred_element_type=F32)
                s0[pl.ds(r0, KC), :] = s
                return jnp.maximum(m, jnp.max(s, axis=0, keepdims=True))
            m = jax.lax.fori_loop(0, S // KC, pass1, jnp.full((1, TQ), -jnp.inf, F32))

            def pass2(c, acc):
                r0 = pl.multiple_of(c * KC, KC)
                p = jnp.exp2(s0[pl.ds(r0, KC), :] - m).astype(BF16)
                vtc = pltpu.bitcast(vt_s[pl.ds(hh, HP // 2), pl.ds(r0, KC)], BF16)
                return acc + jnp.dot(vtc, p, preferred_element_type=F32)
            acc = jax.lax.fori_loop(0, S // KC, pass2, jnp.zeros((HP, TQ), F32))
            o = acc * (1.0 / acc[DH:DH + 1, :])
            ot_s[pl.ds(h0, HP), pl.ds(q0, TQ)] = o.astype(BF16)
            return carry
        jax.lax.fori_loop(0, NCOL, col_body, 0)

    outs = []
    for r in range(len(OCH)):
        cs = slice(sum(OCH[:r]), sum(OCH[:r + 1]))
        a = jnp.dot(wot_s[...], ot_s[:, cs], preferred_element_type=F32)
        ze = jnp.concatenate([z_s[0, cs, :], z_s[2, cs, :]], axis=1)
        zo = jnp.concatenate([z_s[1, cs, :], z_s[3, cs, :]], axis=1)
        e = jax.lax.dot_general(fi_v[0:DHALF, :], ze, NT, preferred_element_type=F32)
        o = jax.lax.dot_general(fi_v[DHALF:, :], zo, NT, preferred_element_type=F32)
        b = jnp.concatenate([e + o, e - o], axis=0)
        g_ = jax.nn.sigmoid(gate_s[0:1, cs])
        o_v[:, cs] = (b + g_ * (a - b)).astype(BF16)
        cpo = pltpu.make_async_copy(o_v.at[:, cs], out_hbm.at[:, cs], osems.at[r])
        cpo.start()
        outs.append(cpo)
    with jax.named_scope('outwait'):
        for cpo in outs:
            cpo.wait()


@jax.jit
def pallas_gated_mix__softmax_full_mha__spectral_gfnet__prompt_kernel(A_x, A_wqkv, A_wo, B_x, B_w_r, B_w_i, gate_w):
    xt = A_x.reshape(S, D).T
    fd, fa, fb, fi = _tables()
    ins = [xt, A_wqkv, A_wo, B_w_r.T, B_w_i.T, gate_w, fd, fa, fb, fi]
    vm = lambda a: pltpu.VMEM(a.shape, a.dtype)
    scratch = [vm(a) for a in ins] + [
        pltpu.VMEM((4, S // 2, 128), jnp.int32), pltpu.VMEM((D, S), BF16), pltpu.VMEM((DP // 2, S), jnp.int32), pltpu.VMEM((DP, S), BF16),
        pltpu.VMEM((D, DP), BF16), pltpu.VMEM((8, S), F32), pltpu.VMEM((2 * D + 16, D), BF16), pltpu.VMEM((D, D), BF16),
    ] + [pltpu.VMEM((4, S, 128), F32) for _ in range(4)] + [
        pltpu.VMEM((32 * 128, 256), BF16), pltpu.VMEM((4, S, 128), BF16), pltpu.VMEM((2, S, 128), jnp.int32),
        pltpu.VMEM((S, TQ), F32), pltpu.VMEM((S // 2, TQ), jnp.int32), pltpu.VMEM((S // 2, TQ), jnp.int32),
        pltpu.VMEM((8 * DH, TQ), F32), pltpu.VMEM((8 * DH, TQ), F32), pltpu.VMEM((8 * DH, TQ), F32), pltpu.VMEM((8 * DH, TQ), F32),
        pltpu.VMEM((D, S), BF16), pltpu.SMEM((1,), jnp.int32),
        pltpu.SemaphoreType.DMA((len(XCH),)), pltpu.SemaphoreType.DMA((9,)), pltpu.SemaphoreType.DMA((len(OCH),)),
    ]
    out = pl.pallas_call(
        _kernel,
        out_shape=jax.ShapeDtypeStruct((D, S), BF16),
        in_specs=[pl.BlockSpec(memory_space=pltpu.HBM)] * len(ins),
        out_specs=pl.BlockSpec(memory_space=pltpu.HBM),
        scratch_shapes=scratch,
        compiler_params=pltpu.CompilerParams(vmem_limit_bytes=110 * 1024 * 1024),
    )(*ins)
    return out.T.reshape(1, S, D)
```

```python
import functools
import numpy as np
import jax
import jax.numpy as jnp
from jax.experimental import pallas as pl
from jax.experimental.pallas import tpu as pltpu

S = 2048
D = 448
DHALF = D // 2
H = 16
DH = 28
HP = 32
DP = H * HP
GW = 4 * DH
DF = D // 2 + 1
TQ = 512
KC = 512
PC = 128
RG = 8
NK = 144
TS = 2
WW = 5
WF = 12
SCHED = (5, 10, 12, 22, 27)
XCH = (256, 256, 512, 1024)
OCH = (512, 512, 512, 384, 128)
NQ = S // TQ
NCOL = NQ * H
F32 = jnp.float32
BF16 = jnp.bfloat16
I32 = jnp.int32
QSCALE = float(DH ** -0.5 * np.log2(np.e))
SMAX = 40.0
VMAX = 2.0 ** 60
TN = (((0,), (0,)), ((), ()))
NT = (((1,), (1,)), ((), ()))


def _real_rep(m):
    return np.block([[m.real, -m.imag], [m.imag, m.real]])


@functools.lru_cache(maxsize=None)
def _tables():
    n = np.arange(DHALF)
    me = np.arange(0, DF, 2)
    mo = np.arange(1, DF, 2)
    fd = np.zeros((2, DHALF, 256))
    fi = np.zeros((2, DHALF, 256))
    for j, mm in enumerate((me, mo)):
        ang = 2 * np.pi * np.outer(n, mm) / D
        c = np.where((mm == 0) | (mm == DF - 1), 1.0, 2.0)
        fd[j, :, :len(mm)] = np.cos(ang)
        fd[j, :, 128:128 + len(mm)] = -np.sin(ang)
        fi[j, :, :len(mm)] = c[None, :] * np.cos(ang) / D
        fi[j, :, 128:128 + len(mm)] = -c[None, :] * np.sin(ang) / D
    b = np.arange(64)
    gc = [np.exp(-2j * np.pi * (np.outer(np.ones(64), b) * c / S + np.outer(b, b) / 64)) for c in range(32)]
    fa = np.stack([_real_rep(g_) for g_ in gc])
    fb = np.transpose(fa, (0, 2, 1)) / S
    bf = lambda a: np.asarray(a, np.float32).astype(jnp.bfloat16)
    return (bf(fd.reshape(2 * DHALF, 256)), bf(fa.reshape(32 * 128, 128)), bf(fb.reshape(32 * 128, 128)),
            bf(fi.reshape(2 * DHALF, 256)))


def _cmulc(z, num, den):
    re, im = z
    num = num % den
    if num == 0:
        return z
    if 4 * num == den:
        return (im, -re)
    if 2 * num == den:
        return (-re, -im)
    if 4 * num == 3 * den:
        return (-im, re)
    c = float(np.cos(2 * np.pi * num / den))
    s_ = float(-np.sin(2 * np.pi * num / den))
    if (8 * num) % den == 0:
        r = abs(c)
        a = re * r
        b = im * r
        if c > 0 and s_ < 0:
            return (a + b, b - a)
        if c < 0 and s_ < 0:
            return (b - a, -(a + b))
        if c < 0 and s_ > 0:
            return (-(a + b), a - b)
        return (a - b, a + b)
    return (re * c - im * s_, re * s_ + im * c)


def _add(a, b):
    return (a[0] + b[0], a[1] + b[1])


def _sub(a, b):
    return (a[0] - b[0], a[1] - b[1])


def _fft4(x, sign):
    t0, t1 = _add(x[0], x[2]), _sub(x[0], x[2])
    t2, t3 = _add(x[1], x[3]), _sub(x[1], x[3])
    y0, y2 = _add(t0, t2), _sub(t0, t2)
    ym = (t1[0] + t3[1], t1[1] - t3[0])
    yp = (t1[0] - t3[1], t1[1] + t3[0])
    return [y0, ym, y2, yp] if sign > 0 else [y0, yp, y2, ym]


def _fft8(x, sign):
    e = _fft4(x[0::2], sign)
    o = _fft4(x[1::2], sign)
    o = [_cmulc(o[k], sign * k, 8) for k in range(4)]
    return [_add(e[k], o[k]) for k in range(4)] + [_sub(e[k], o[k]) for k in range(4)]


def _paced(x, tie):
    if tie.dtype != x.dtype:
        return jnp.where(tie != tie, pltpu.bitcast(tie, x.dtype), x)
    return jnp.where(tie != tie, tie, x)


def _kernel(xt_hbm, w_hbm, wo_hbm, wr_hbm, wi_hbm, gw_hbm, fd_hbm, fa_hbm, fb_hbm, fi_hbm,
            out_hbm,
            xt_v, w_v, wo_v, wr_v, wi_v, gw_v, fd_v, fa_v, fb_v, fi_v,
            k_s, qt_s, vt_s, ot_s, wot_s, gate_s, wt_s, wvt_s,
            x_s, p_s, u_s, q_s, yb_s, z_s, wu_s,
            s0, p0, p1, qb0, qb1, qb2, qb3, o_v, flag_s, xsems, sems, osems):
    P = functools.partial
    NX = len(XCH)
    xoff = [sum(XCH[:j]) for j in range(NX)]
    xcp = [pltpu.make_async_copy(xt_hbm.at[:, pl.ds(xoff[j], XCH[j])], xt_v.at[:, pl.ds(xoff[j], XCH[j])], xsems.at[j])
           for j in range(NX)]
    names = ['fd', 'w', 'gw', 'wr', 'wi', 'fa', 'fb', 'wo', 'fi']
    srcs = [fd_hbm, w_hbm, gw_hbm, wr_hbm, wi_hbm, fa_hbm, fb_hbm, wo_hbm, fi_hbm]
    dsts = [fd_v, w_v, gw_v, wr_v, wi_v, fa_v, fb_v, wo_v, fi_v]
    cp = {n: pltpu.make_async_copy(s, d, sems.at[i]) for i, (n, s, d) in enumerate(zip(names, srcs, dsts))}
    xcp[0].start()
    cp['fd'].start()
    for c in xcp[1:]:
        c.start()
    cp['w'].start()
    cp['fd'].wait()

    for j in range(NX):
        xcp[j].wait()
        cs = pl.ds(xoff[j], XCH[j])
        x1 = xt_v[:DHALF, cs].astype(F32)
        x2 = xt_v[DHALF:, cs].astype(F32)
        et = (x1 + x2).astype(BF16)
        ot = (x1 - x2).astype(BF16)
        xe = jax.lax.dot_general(et, fd_v[0:DHALF, :], TN, preferred_element_type=F32)
        x_s[0, cs, :] = xe[:, :128]
        x_s[2, cs, :] = xe[:, 128:]
        xo = jax.lax.dot_general(ot, fd_v[DHALF:, :], TN, preferred_element_type=F32)
        x_s[1, cs, :] = xo[:, :128]
        x_s[3, cs, :] = xo[:, 128:]
    cp['gw'].start()
    cp['w'].wait()
    cp['gw'].wait()
    for n in ['wr', 'wi', 'fa', 'fb', 'wo', 'fi']:
        cp[n].start()
    wt = w_v[...].T
    gw = gw_v[...].reshape(1, D)
    wt_s[...] = jnp.concatenate([wt[0:2 * D], gw, jnp.zeros((15, D), BF16)], axis=0)
    wvt_s[...] = wt[2 * D:]

    def w_task(j, t, tie):
        ref = (wr_v, wi_v)[j]
        cs = pl.ds(t * 512, 512)
        u = pltpu.bitcast(ref[0:DHALF, cs], I32)
        last = jax.lax.shift_right_logical(pltpu.bitcast(ref[DHALF:DF, cs].astype(F32), I32), 16)
        up = jnp.concatenate([u, last, jnp.zeros((15, 512), I32)], axis=0)
        wu_s[j, cs, :] = up.T

    def load_c(ref, lt, rows, tie):
        xs = [(ref[lt, pl.ds(r, RG), :], ref[2 + lt, pl.ds(r, RG), :]) for r in rows]
        return [(_paced(xs[0][0], tie), xs[0][1])] + xs[1:]

    def p1_task(a0, lt, r0, tie):
        ys = _fft4(load_c(x_s, lt, [512 * a1 + 64 * a0 + r0 for a1 in range(4)], tie), 1)
        for c0 in range(4):
            y = _cmulc(ys[c0], a0 * c0, 32)
            p_s[lt, pl.ds(512 * c0 + 64 * a0 + r0, RG), :] = y[0]
            p_s[2 + lt, pl.ds(512 * c0 + 64 * a0 + r0, RG), :] = y[1]

    def p2_task(c0, lt, r0, tie):
        ys = _fft8(load_c(p_s, lt, [512 * c0 + 64 * a0 + r0 for a0 in range(8)], tie), 1)
        for c1 in range(8):
            c = c0 + 4 * c1
            yb_s[pl.ds(128 * c + r0, RG), pl.ds(128 * lt, 128)] = ys[c1][0].astype(BF16)
            yb_s[pl.ds(128 * c + 64 + r0, RG), pl.ds(128 * lt, 128)] = ys[c1][1].astype(BF16)

    def smx_task(c, tie):
        hi = jnp.int32(-65536)
        xk = jnp.dot(fa_v[c * 128:(c + 1) * 128, :], yb_s[c * 128:(c + 1) * 128, :], preferred_element_type=F32)
        xr, xi = xk[:64], xk[64:]
        ur = wu_s[0, pl.ds(c, 64, stride=32), :]
        ui = wu_s[1, pl.ds(c, 64, stride=32), :]
        wr = jnp.concatenate([pltpu.bitcast(ur << 16, F32), pltpu.bitcast(ur & hi, F32)], axis=1)
        wi = jnp.concatenate([pltpu.bitcast(ui << 16, F32), pltpu.bitcast(ui & hi, F32)], axis=1)
        y = jnp.concatenate([xr * wr - xi * wi, xr * wi + xi * wr], axis=0).astype(BF16)
        u = jnp.dot(fb_v[c * 128:(c + 1) * 128, :], y, preferred_element_type=F32)
        u_s[0, pl.ds(64 * c, 64), :] = u[:64, :128]
        u_s[1, pl.ds(64 * c, 64), :] = u[:64, 128:]
        u_s[2, pl.ds(64 * c, 64), :] = u[64:, :128]
        u_s[3, pl.ds(64 * c, 64), :] = u[64:, 128:]

    def ip2_task(c0, lt, r0, tie):
        ys = _fft8(load_c(u_s, lt, [64 * (c0 + 4 * c1) + r0 for c1 in range(8)], tie), -1)
        for a0 in range(8):
            y = _cmulc(ys[a0], -a0 * c0, 32)
            q_s[lt, pl.ds(512 * c0 + 64 * a0 + r0, RG), :] = y[0]
            q_s[2 + lt, pl.ds(512 * c0 + 64 * a0 + r0, RG), :] = y[1]

    def ip1_task(a0, lt, r0, tie):
        ys = _fft4(load_c(q_s, lt, [512 * c0 + 64 * a0 + r0 for c0 in range(4)], tie), -1)
        for a1 in range(4):
            z_s[lt, pl.ds(512 * a1 + 64 * a0 + r0, RG), :] = ys[a1][0].astype(BF16)
            z_s[2 + lt, pl.ds(512 * a1 + 64 * a0 + r0, RG), :] = ys[a1][1].astype(BF16)

    def wo_task(tie):
        wof = wo_v[...].astype(F32)
        pieces = []
        for h in range(H):
            pieces += [wof[DH * h:DH * (h + 1)], jnp.zeros((HP - DH, D), F32)]
        wot_s[...] = jnp.concatenate(pieces, axis=0).astype(BF16).T

    rr = range(0, 64, RG)
    t_p1 = [P(p1_task, a0, lt, r0) for lt in range(2) for r0 in rr for a0 in range(8)]
    t_p2 = [P(p2_task, c0, lt, r0) for lt in range(2) for r0 in rr for c0 in range(4)]
    t_w = [P(w_task, j, t) for j in range(2) for t in range(4)]
    t_smx = [P(smx_task, c) for c in range(32)]
    t_ip2 = [P(ip2_task, c0, lt, r0) for lt in range(2) for r0 in rr for c0 in range(4)]
    t_ip1 = [P(ip1_task, a0, lt, r0) for lt in range(2) for r0 in rr for a0 in range(8)]

    def share(tasks, a, b, j):
        if not a <= j < b:
            return []
        return tasks[len(tasks) * (j - a) // (b - a):len(tasks) * (j - a + 1) // (b - a)]

    def side_tasks(j, res):
        pa, pb, we, se, ie = SCHED
        tasks = (share(t_p1, 0, pa, j) + share(t_p2, pa, pb, j) + share(t_w, WW, we, j) + share(t_smx, WF, se, j)
                 + share(t_ip2, se, ie, j) + share(t_ip1, ie, 32, j) + share([wo_task], 30, 31, j))
        nr = res.shape[0] // 8
        for i, t in enumerate(tasks):
            r = nr * i // len(tasks) * 8
            t(res[r:r + 8, 0:128])

    nq = [jnp.zeros((1, PC), F32) for _ in range(4)]
    nk = [jnp.zeros((1, PC), F32) for _ in range(4)]
    for j in range(S // PC):
        if j == WW:
            cp['wr'].wait()
            cp['wi'].wait()
        if j == WF:
            for n in ['fa', 'fb', 'wo', 'fi']:
                cp[n].wait()
        cs = pl.ds(j * PC, PC)
        qk = jnp.dot(wt_s[...], xt_v[:, cs], preferred_element_type=F32)
        gate_s[:, cs] = jnp.broadcast_to(qk[2 * D:2 * D + 1, :], (8, PC))
        q = qk[0:D] * QSCALE
        qt_s[:, cs] = q.astype(BF16)
        for g in range(4):
            qg = q[GW * g:GW * (g + 1)]
            nq[g] = jnp.maximum(nq[g], jnp.sum(qg * qg, axis=0, keepdims=True))
            kg = qk[D + GW * g:D + GW * (g + 1)]
            nk[g] = jnp.maximum(nk[g], jnp.sum(kg * kg, axis=0, keepdims=True))
            kg = jnp.concatenate([kg, jnp.zeros((128 - GW, PC), F32)], axis=0)
            k_s[g, pl.ds(j * PC // 2, PC // 2), :] = pltpu.bitcast(kg.astype(BF16).T, I32)
        side_tasks(j, qk)
    vmax = jnp.zeros((8, PC), F32)
    for j in range(S // PC):
        cs = pl.ds(j * PC, PC)
        vt = jnp.dot(wvt_s[...], xt_v[:, cs], preferred_element_type=F32)
        tail = jnp.concatenate([jnp.ones((1, PC), F32), jnp.zeros((HP - DH - 1, PC), F32)], axis=0)
        pieces = []
        for h in range(H):
            pieces += [vt[DH * h:DH * (h + 1)], tail]
        vt_s[:, cs] = pltpu.bitcast(jnp.concatenate(pieces, axis=0).astype(BF16), I32)
        vmax = jnp.maximum(vmax, jnp.max(jnp.abs(vt).reshape(D // 8, 8, PC), axis=0))
        side_tasks(16 + j, vt)
    bound2 = jnp.max(nq[0]) * jnp.max(nk[0])
    for g in range(1, 4):
        bound2 = jnp.maximum(bound2, jnp.max(nq[g]) * jnp.max(nk[g]))
    safe = jnp.logical_and(bound2 * 1.02 <= SMAX * SMAX, jnp.max(vmax) <= VMAX)
    flag_s[0] = jnp.where(safe, 0, 1).astype(I32)

    def prep_q(col, sub, qb=None):
        q0 = pl.multiple_of((col // H) * TQ, TQ)
        r0 = pl.multiple_of(((col % H) // 4) * GW, 16)
        r = jax.lax.broadcasted_iota(I32, (GW, TQ), 0)
        qg = qt_s[pl.ds(r0, GW), pl.ds(q0, TQ)].astype(F32)
        qm = jnp.where((r >= sub * DH) & (r < sub * DH + DH), qg, 0.0).astype(BF16)
        if qb is not None:
            for d in range(DH):
                qb[8 * d:8 * d + 8, :] = jnp.broadcast_to(qg[DH * sub + d:DH * sub + d + 1, :], (8, TQ))
        return jnp.concatenate([qm, jnp.zeros((128 - GW, TQ), BF16)], axis=0)

    KM = S - NK

    def tie_row(jb, d):
        return ((jb * DH + d) * (KM // 8)) // (NK // 16 * DH)

    def vpu_block(jb, g, sub, qb, pA, ss):
        kw = k_s[g, pl.ds(KM // 2 + 8 * jb, 8), :]
        acc0 = acc1 = None
        for d in range(DH):
            lane = DH * sub + d
            kbw = jnp.broadcast_to(kw[:, lane:lane + 1], (8, 128))
            if d % TS == 0:
                r = tie_row(jb, d)
                cc, r = r // (KC // 8), r % (KC // 8)
                kbw = _paced(kbw, ss[cc][8 * r:8 * r + 8, 128 * (d % 4):128 * (d % 4) + 128])
            kb0 = pltpu.bitcast(kbw << 16, F32)
            kb1 = pltpu.bitcast(kbw & jnp.int32(-65536), F32)
            q = qb[8 * d:8 * d + 8, :]
            t0 = jnp.concatenate([kb0] * (TQ // 128), axis=1) * q
            t1 = jnp.concatenate([kb1] * (TQ // 128), axis=1) * q
            acc0 = t0 if acc0 is None else acc0 + t0
            acc1 = t1 if acc1 is None else acc1 + t1
        e0 = pltpu.bitcast(jnp.exp2(acc0).astype(BF16).astype(F32), I32)
        e1 = pltpu.bitcast(jnp.exp2(acc1).astype(BF16).astype(F32), I32)
        pA[pl.ds(KM // 2 + 8 * jb, 8), :] = jax.lax.shift_right_logical(e0, 16) | e1

    def stages(colA, sub, qb, pA, colB, pB):
        KH = KC // 2
        if colA is not None:
            g = (colA % H) // 4
            qm = prep_q(colA, sub, qb)
        if colB is not None:
            h0 = pl.multiple_of((colB % H) * HP, HP)
            hh = pl.multiple_of((colB % H) * (HP // 2), HP // 2)
            q0 = pl.multiple_of((colB // H) * TQ, TQ)
            acc = jnp.zeros((HP, TQ), F32)
        ss = []
        for c in range(S // KC):
            if colA is not None:
                n = min(KC, KM - c * KC)
                kc = pltpu.bitcast(k_s[g, pl.ds(c * KH, n // 2), :], BF16)
                s = jnp.dot(kc, qm, preferred_element_type=F32)
                pA[pl.ds(c * KH, n // 2), :] = pltpu.bitcast(jnp.exp2(s).astype(BF16), I32)
                ss.append(s)
                for jb in range(NK // 16):
                    if tie_row(jb, DH - 1) // (KC // 8) == c:
                        vpu_block(jb, g, sub, qb, pA, ss)
            if colB is not None:
                p = pltpu.bitcast(pB[pl.ds(c * KH, KH), :], BF16)
                vtc = pltpu.bitcast(vt_s[pl.ds(hh, HP // 2), pl.ds(c * KC, KC)], BF16)
                acc = acc + jnp.dot(vtc, p, preferred_element_type=F32)
        if colB is not None:
            o = acc * (1.0 / acc[DH:DH + 1, :])
            ot_s[pl.ds(h0, HP), pl.ds(q0, TQ)] = o.astype(BF16)

    def pair(c, c4, qbs):
        stages(c + 1, (c4 + 1) % 4, qbs[0], p1, c, p0)
        stages(c + 2, (c4 + 2) % 4, qbs[1], p0, c + 1, p1)

    stages(0, 0, qb0, p0, None, None)

    def body(i, carry):
        pair(4 * i, 0, (qb1, qb0))
        pair(4 * i + 2, 2, (qb3, qb2))
        return carry
    jax.lax.fori_loop(0, NCOL // 4 - 1, body, 0)
    pair(NCOL - 4, 0, (qb1, qb0))
    stages(NCOL - 1, 3, qb1, p1, NCOL - 2, p0)
    stages(None, None, None, None, NCOL - 1, p1)

    @pl.when(flag_s[0] == 1)
    def _():
        def col_body(col, carry):
            g = (col % H) // 4
            qm = prep_q(col, col % 4)
            h0 = pl.multiple_of((col % H) * HP, HP)
            hh = pl.multiple_of((col % H) * (HP // 2), HP // 2)
            q0 = pl.multiple_of((col // H) * TQ, TQ)

            def pass1(c, m):
                r0 = pl.multiple_of(c * KC, KC)
                kc = pltpu.bitcast(k_s[g, pl.ds(pl.multiple_of(c * (KC // 2), KC // 2), KC // 2), :], BF16)
                s = jnp.dot(kc, qm, preferred_element_type=F32)
                s0[pl.ds(r0, KC), :] = s
                return jnp.maximum(m, jnp.max(s, axis=0, keepdims=True))
            m = jax.lax.fori_loop(0, S // KC, pass1, jnp.full((1, TQ), -jnp.inf, F32))

            def pass2(c, acc):
                r0 = pl.multiple_of(c * KC, KC)
                p = jnp.exp2(s0[pl.ds(r0, KC), :] - m).astype(BF16)
                vtc = pltpu.bitcast(vt_s[pl.ds(hh, HP // 2), pl.ds(r0, KC)], BF16)
                return acc + jnp.dot(vtc, p, preferred_element_type=F32)
            acc = jax.lax.fori_loop(0, S // KC, pass2, jnp.zeros((HP, TQ), F32))
            o = acc * (1.0 / acc[DH:DH + 1, :])
            ot_s[pl.ds(h0, HP), pl.ds(q0, TQ)] = o.astype(BF16)
            return carry
        jax.lax.fori_loop(0, NCOL, col_body, 0)

    outs = []
    for r in range(len(OCH)):
        cs = slice(sum(OCH[:r]), sum(OCH[:r + 1]))
        a = jnp.dot(wot_s[...], ot_s[:, cs], preferred_element_type=F32)
        ze = jnp.concatenate([z_s[0, cs, :], z_s[2, cs, :]], axis=1)
        zo = jnp.concatenate([z_s[1, cs, :], z_s[3, cs, :]], axis=1)
        e = jax.lax.dot_general(fi_v[0:DHALF, :], ze, NT, preferred_element_type=F32)
        o = jax.lax.dot_general(fi_v[DHALF:, :], zo, NT, preferred_element_type=F32)
        b = jnp.concatenate([e + o, e - o], axis=0)
        g_ = jax.nn.sigmoid(gate_s[0:1, cs])
        o_v[:, cs] = (b + g_ * (a - b)).astype(BF16)
        cpo = pltpu.make_async_copy(o_v.at[:, cs], out_hbm.at[:, cs], osems.at[r])
        cpo.start()
        outs.append(cpo)
    for cpo in outs:
        cpo.wait()


@jax.jit
def pallas_gated_mix__softmax_full_mha__spectral_gfnet__prompt_kernel(A_x, A_wqkv, A_wo, B_x, B_w_r, B_w_i, gate_w):
    del B_x
    xt = A_x.reshape(S, D).T
    fd, fa, fb, fi = _tables()
    ins = [xt, A_wqkv, A_wo, B_w_r.T, B_w_i.T, gate_w, fd, fa, fb, fi]
    vm = lambda a: pltpu.VMEM(a.shape, a.dtype)
    scratch = [vm(a) for a in ins] + [
        pltpu.VMEM((4, S // 2, 128), I32),
        pltpu.VMEM((D, S), BF16),
        pltpu.VMEM((DP // 2, S), I32),
        pltpu.VMEM((DP, S), BF16),
        pltpu.VMEM((D, DP), BF16),
        pltpu.VMEM((8, S), F32),
        pltpu.VMEM((2 * D + 16, D), BF16),
        pltpu.VMEM((D, D), BF16),
    ] + [pltpu.VMEM((4, S, 128), F32) for _ in range(4)] + [
        pltpu.VMEM((32 * 128, 256), BF16), pltpu.VMEM((4, S, 128), BF16), pltpu.VMEM((2, S, 128), I32),
        pltpu.VMEM((S, TQ), F32), pltpu.VMEM((S // 2, TQ), I32), pltpu.VMEM((S // 2, TQ), I32),
    ] + [pltpu.VMEM((8 * DH, TQ), F32) for _ in range(4)] + [
        pltpu.VMEM((D, S), BF16), pltpu.SMEM((1,), I32),
        pltpu.SemaphoreType.DMA((len(XCH),)), pltpu.SemaphoreType.DMA((9,)), pltpu.SemaphoreType.DMA((len(OCH),)),
    ]
    out = pl.pallas_call(
        _kernel,
        out_shape=jax.ShapeDtypeStruct((D, S), BF16),
        in_specs=[pl.BlockSpec(memory_space=pltpu.HBM)] * len(ins),
        out_specs=pl.BlockSpec(memory_space=pltpu.HBM),
        scratch_shapes=scratch,
        compiler_params=pltpu.CompilerParams(vmem_limit_bytes=110 * 1024 * 1024),
    )(*ins)
    return out.T.reshape(1, S, D)
```

```python
import functools
import numpy as np
import jax
import jax.numpy as jnp
from jax.experimental import pallas as pl
from jax.experimental.pallas import tpu as pltpu

S = 2048
D = 448
DHALF = D // 2
H = 16
DH = 28
HP = 32
DP = H * HP
GW = 4 * DH
DF = D // 2 + 1
TQ = 512
KC = 512
PC = 128
RG = 8
NK = 144
TS = 2
WW = 5
WF = 12
SCHED = (5, 9, 12, 12, 20, 22, 27)
XCH = (256, 256, 512, 1024)
OCH = (512, 512, 512, 384, 128)
NQ = S // TQ
NCOL = NQ * H
F32 = jnp.float32
BF16 = jnp.bfloat16
I32 = jnp.int32
QSCALE = float(DH ** -0.5 * np.log2(np.e))
SMAX = 40.0
VMAX = 2.0 ** 60
TN = (((0,), (0,)), ((), ()))
NT = (((1,), (1,)), ((), ()))


def _real_rep(m):
    return np.block([[m.real, -m.imag], [m.imag, m.real]])


@functools.lru_cache(maxsize=None)
def _tables():
    n = np.arange(DHALF)
    me = np.arange(0, DF, 2)
    mo = np.arange(1, DF, 2)
    fd = np.zeros((2, DHALF, 256))
    fi = np.zeros((2, DHALF, 256))
    for j, mm in enumerate((me, mo)):
        ang = 2 * np.pi * np.outer(n, mm) / D
        c = np.where((mm == 0) | (mm == DF - 1), 1.0, 2.0)
        fd[j, :, :len(mm)] = np.cos(ang)
        fd[j, :, 128:128 + len(mm)] = -np.sin(ang)
        fi[j, :, :len(mm)] = c[None, :] * np.cos(ang) / D
        fi[j, :, 128:128 + len(mm)] = -c[None, :] * np.sin(ang) / D
    b = np.arange(64)
    gc = [np.exp(-2j * np.pi * (np.outer(np.ones(64), b) * c / S + np.outer(b, b) / 64)) for c in range(32)]
    fa = np.stack([_real_rep(g_) for g_ in gc])
    fb = np.transpose(fa, (0, 2, 1)) / S
    bf = lambda a: np.asarray(a, np.float32).astype(jnp.bfloat16)
    return (bf(fd.reshape(2 * DHALF, 256)), bf(fa.reshape(32 * 128, 128)), bf(fb.reshape(32 * 128, 128)),
            bf(fi.reshape(2 * DHALF, 256)))


def _cmulc(z, num, den):
    re, im = z
    num = num % den
    if num == 0:
        return z
    if 4 * num == den:
        return (im, -re)
    if 2 * num == den:
        return (-re, -im)
    if 4 * num == 3 * den:
        return (-im, re)
    c = float(np.cos(2 * np.pi * num / den))
    s_ = float(-np.sin(2 * np.pi * num / den))
    if (8 * num) % den == 0:
        r = abs(c)
        a = re * r
        b = im * r
        if c > 0 and s_ < 0:
            return (a + b, b - a)
        if c < 0 and s_ < 0:
            return (b - a, -(a + b))
        if c < 0 and s_ > 0:
            return (-(a + b), a - b)
        return (a - b, a + b)
    return (re * c - im * s_, re * s_ + im * c)


def _add(a, b):
    return (a[0] + b[0], a[1] + b[1])


def _sub(a, b):
    return (a[0] - b[0], a[1] - b[1])


def _fft4(x, sign):
    t0, t1 = _add(x[0], x[2]), _sub(x[0], x[2])
    t2, t3 = _add(x[1], x[3]), _sub(x[1], x[3])
    y0, y2 = _add(t0, t2), _sub(t0, t2)
    ym = (t1[0] + t3[1], t1[1] - t3[0])
    yp = (t1[0] - t3[1], t1[1] + t3[0])
    return [y0, ym, y2, yp] if sign > 0 else [y0, yp, y2, ym]


def _fft8(x, sign):
    e = _fft4(x[0::2], sign)
    o = _fft4(x[1::2], sign)
    o = [_cmulc(o[k], sign * k, 8) for k in range(4)]
    return [_add(e[k], o[k]) for k in range(4)] + [_sub(e[k], o[k]) for k in range(4)]


def _paced(x, tie):
    if tie.dtype != x.dtype:
        return jnp.where(tie != tie, pltpu.bitcast(tie, x.dtype), x)
    return jnp.where(tie != tie, tie, x)


def _kernel(xt_hbm, w_hbm, wo_hbm, wr_hbm, wi_hbm, gw_hbm, fd_hbm, fa_hbm, fb_hbm, fi_hbm,
            out_hbm,
            xt_v, w_v, wo_v, wr_v, wi_v, gw_v, fd_v, fa_v, fb_v, fi_v,
            k_s, qt_s, vt_s, ot_s, wot_s, gate_s, wt_s, wvt_s,
            x_s, p_s, u_s, q_s, yb_s, z_s, wu_s,
            s0, p0, p1, qb0, qb1, qb2, qb3, l_s, o_v, flag_s, xsems, sems, osems):
    P = functools.partial
    NX = len(XCH)
    xoff = [sum(XCH[:j]) for j in range(NX)]
    xcp = [pltpu.make_async_copy(xt_hbm.at[:, pl.ds(xoff[j], XCH[j])], xt_v.at[:, pl.ds(xoff[j], XCH[j])], xsems.at[j])
           for j in range(NX)]
    names = ['fd', 'w', 'gw', 'wr', 'wi', 'fa', 'fb', 'wo', 'fi']
    srcs = [fd_hbm, w_hbm, gw_hbm, wr_hbm, wi_hbm, fa_hbm, fb_hbm, wo_hbm, fi_hbm]
    dsts = [fd_v, w_v, gw_v, wr_v, wi_v, fa_v, fb_v, wo_v, fi_v]
    cp = {n: pltpu.make_async_copy(s, d, sems.at[i]) for i, (n, s, d) in enumerate(zip(names, srcs, dsts))}
    xcp[0].start()
    cp['fd'].start()
    for c in xcp[1:]:
        c.start()
    cp['w'].start()
    cp['fd'].wait()

    for j in range(NX):
        xcp[j].wait()
        cs = pl.ds(xoff[j], XCH[j])
        x1 = xt_v[:DHALF, cs].astype(F32)
        x2 = xt_v[DHALF:, cs].astype(F32)
        et = (x1 + x2).astype(BF16)
        ot = (x1 - x2).astype(BF16)
        xe = jax.lax.dot_general(et, fd_v[0:DHALF, :], TN, preferred_element_type=F32)
        x_s[0, cs, :] = xe[:, :128]
        x_s[2, cs, :] = xe[:, 128:]
        xo = jax.lax.dot_general(ot, fd_v[DHALF:, :], TN, preferred_element_type=F32)
        x_s[1, cs, :] = xo[:, :128]
        x_s[3, cs, :] = xo[:, 128:]
    cp['gw'].start()
    cp['w'].wait()
    cp['gw'].wait()
    for n in ['wr', 'wi', 'fa', 'fb', 'wo', 'fi']:
        cp[n].start()
    wt = w_v[...].T
    gw = gw_v[...].reshape(1, D)
    wt_s[...] = jnp.concatenate([wt[0:2 * D], gw, jnp.zeros((15, D), BF16)], axis=0)
    wvt_s[...] = wt[2 * D:]

    def w_task(j, t, tie):
        ref = (wr_v, wi_v)[j]
        cs = pl.ds(t * 512, 512)
        u = pltpu.bitcast(ref[0:DHALF, cs], I32)
        last = jax.lax.shift_right_logical(pltpu.bitcast(ref[DHALF:DF, cs].astype(F32), I32), 16)
        up = jnp.concatenate([u, last, jnp.zeros((15, 512), I32)], axis=0)
        wu_s[j, cs, :] = up.T

    def load_c(ref, lt, rows, tie):
        xs = [(ref[lt, pl.ds(r, RG), :], ref[2 + lt, pl.ds(r, RG), :]) for r in rows]
        return [(_paced(xs[0][0], tie), xs[0][1])] + xs[1:]

    def p1_task(a0, lt, r0, tie):
        ys = _fft4(load_c(x_s, lt, [512 * a1 + 64 * a0 + r0 for a1 in range(4)], tie), 1)
        for c0 in range(4):
            y = _cmulc(ys[c0], a0 * c0, 32)
            p_s[lt, pl.ds(512 * c0 + 64 * a0 + r0, RG), :] = y[0]
            p_s[2 + lt, pl.ds(512 * c0 + 64 * a0 + r0, RG), :] = y[1]

    def p2_task(c0, lt, r0, tie):
        ys = _fft8(load_c(p_s, lt, [512 * c0 + 64 * a0 + r0 for a0 in range(8)], tie), 1)
        for c1 in range(8):
            c = c0 + 4 * c1
            yb_s[pl.ds(128 * c + r0, RG), pl.ds(128 * lt, 128)] = ys[c1][0].astype(BF16)
            yb_s[pl.ds(128 * c + 64 + r0, RG), pl.ds(128 * lt, 128)] = ys[c1][1].astype(BF16)

    def smx_task(c, tie):
        hi = jnp.int32(-65536)
        xk = jnp.dot(fa_v[c * 128:(c + 1) * 128, :], yb_s[c * 128:(c + 1) * 128, :], preferred_element_type=F32)
        xr, xi = xk[:64], xk[64:]
        ur = wu_s[0, pl.ds(c, 64, stride=32), :]
        ui = wu_s[1, pl.ds(c, 64, stride=32), :]
        wr = jnp.concatenate([pltpu.bitcast(ur << 16, F32), pltpu.bitcast(ur & hi, F32)], axis=1)
        wi = jnp.concatenate([pltpu.bitcast(ui << 16, F32), pltpu.bitcast(ui & hi, F32)], axis=1)
        y = jnp.concatenate([xr * wr - xi * wi, xr * wi + xi * wr], axis=0).astype(BF16)
        u = jnp.dot(fb_v[c * 128:(c + 1) * 128, :], y, preferred_element_type=F32)
        u_s[0, pl.ds(64 * c, 64), :] = u[:64, :128]
        u_s[1, pl.ds(64 * c, 64), :] = u[:64, 128:]
        u_s[2, pl.ds(64 * c, 64), :] = u[64:, :128]
        u_s[3, pl.ds(64 * c, 64), :] = u[64:, 128:]

    def ip2_task(c0, lt, r0, tie):
        ys = _fft8(load_c(u_s, lt, [64 * (c0 + 4 * c1) + r0 for c1 in range(8)], tie), -1)
        for a0 in range(8):
            y = _cmulc(ys[a0], -a0 * c0, 32)
            q_s[lt, pl.ds(512 * c0 + 64 * a0 + r0, RG), :] = y[0]
            q_s[2 + lt, pl.ds(512 * c0 + 64 * a0 + r0, RG), :] = y[1]

    def ip1_task(a0, lt, r0, tie):
        ys = _fft4(load_c(q_s, lt, [512 * c0 + 64 * a0 + r0 for c0 in range(4)], tie), -1)
        for a1 in range(4):
            z_s[lt, pl.ds(512 * a1 + 64 * a0 + r0, RG), :] = ys[a1][0].astype(BF16)
            z_s[2 + lt, pl.ds(512 * a1 + 64 * a0 + r0, RG), :] = ys[a1][1].astype(BF16)

    def wo_task(tie):
        wof = wo_v[...].astype(F32)
        pieces = []
        for h in range(H):
            pieces += [wof[DH * h:DH * (h + 1)], jnp.zeros((HP - DH, D), F32)]
        wot_s[...] = jnp.concatenate(pieces, axis=0).astype(BF16).T

    rr = range(0, 64, RG)
    t_p1 = [P(p1_task, a0, lt, r0) for lt in range(2) for r0 in rr for a0 in range(8)]
    t_p2 = [P(p2_task, c0, lt, r0) for lt in range(2) for r0 in rr for c0 in range(4)]
    t_w = [P(w_task, j, t) for j in range(2) for t in range(4)]
    t_smx = [P(smx_task, c) for c in range(32)]
    t_ip2 = [P(ip2_task, c0, lt, r0) for lt in range(2) for r0 in rr for c0 in range(4)]
    t_ip1 = [P(ip1_task, a0, lt, r0) for lt in range(2) for r0 in rr for a0 in range(8)]

    def share(tasks, a, b, j):
        if not a <= j < b:
            return []
        return tasks[len(tasks) * (j - a) // (b - a):len(tasks) * (j - a + 1) // (b - a)]

    def side_tasks(j, res):
        pa, pb, we, ss_, se, i0, ie = SCHED
        tasks = (share(t_p1, 0, pa, j) + share(t_p2, pa, pb, j) + share(t_w, WW, we, j) + share(t_smx, ss_, se, j)
                 + share(t_ip2, i0, ie, j) + share(t_ip1, ie, 32, j) + share([wo_task], 30, 31, j))
        nr = res.shape[0] // 8
        for i, t in enumerate(tasks):
            r = nr * i // len(tasks) * 8
            t(res[r:r + 8, 0:128])

    nq = [jnp.zeros((1, PC), F32) for _ in range(4)]
    nk = [jnp.zeros((1, PC), F32) for _ in range(4)]
    for j in range(S // PC):
        if j == WW:
            cp['wr'].wait()
            cp['wi'].wait()
        if j == WF:
            for n in ['fa', 'fb', 'wo', 'fi']:
                cp[n].wait()
        cs = pl.ds(j * PC, PC)
        qk = jnp.dot(wt_s[...], xt_v[:, cs], preferred_element_type=F32)
        gate_s[:, cs] = jnp.broadcast_to(qk[2 * D:2 * D + 1, :], (8, PC))
        q = qk[0:D] * QSCALE
        qt_s[:, cs] = q.astype(BF16)
        for g in range(4):
            qg = q[GW * g:GW * (g + 1)]
            nq[g] = jnp.maximum(nq[g], jnp.sum(qg * qg, axis=0, keepdims=True))
            kg = qk[D + GW * g:D + GW * (g + 1)]
            nk[g] = jnp.maximum(nk[g], jnp.sum(kg * kg, axis=0, keepdims=True))
            kg = jnp.concatenate([kg, jnp.zeros((128 - GW, PC), F32)], axis=0)
            k_s[g, pl.ds(j * PC // 2, PC // 2), :] = pltpu.bitcast(kg.astype(BF16).T, I32)
        side_tasks(j, qk)
    vmax = jnp.zeros((8, PC), F32)
    for j in range(S // PC):
        cs = pl.ds(j * PC, PC)
        vt = jnp.dot(wvt_s[...], xt_v[:, cs], preferred_element_type=F32)
        tail = jnp.concatenate([jnp.ones((1, PC), F32), jnp.zeros((HP - DH - 1, PC), F32)], axis=0)
        pieces = []
        for h in range(H):
            pieces += [vt[DH * h:DH * (h + 1)], tail]
        vt_s[:, cs] = pltpu.bitcast(jnp.concatenate(pieces, axis=0).astype(BF16), I32)
        vmax = jnp.maximum(vmax, jnp.max(jnp.abs(vt).reshape(D // 8, 8, PC), axis=0))
        side_tasks(16 + j, vt)
    bound2 = jnp.max(nq[0]) * jnp.max(nk[0])
    for g in range(1, 4):
        bound2 = jnp.maximum(bound2, jnp.max(nq[g]) * jnp.max(nk[g]))
    safe = jnp.logical_and(bound2 * 1.02 <= SMAX * SMAX, jnp.max(vmax) <= VMAX)
    flag_s[0] = jnp.where(safe, 0, 1).astype(I32)

    def prep_q(col, sub, qb=None):
        q0 = pl.multiple_of((col >> 4) * TQ, TQ)
        r0 = pl.multiple_of(((col >> 2) & 3) * GW, 16)
        if isinstance(sub, int):
            lo, hi = sub * DH // 16 * 16, -(-(sub + 1) * DH // 16) * 16
        else:
            lo, hi = 0, GW
        r = jax.lax.broadcasted_iota(I32, (hi - lo, TQ), 0) + lo
        qg = qt_s[pl.ds(pl.multiple_of(r0 + lo, 16), hi - lo), pl.ds(q0, TQ)].astype(F32)
        qm = jnp.where((r >= sub * DH) & (r < sub * DH + DH), qg, 0.0).astype(BF16)
        if qb is not None:
            for d in range(DH):
                row = DH * sub + d - lo
                qb[8 * d:8 * d + 8, :] = jnp.broadcast_to(qg[row:row + 1, :], (8, TQ))
        pieces = [jnp.zeros((lo, TQ), BF16)] if lo else []
        return jnp.concatenate(pieces + [qm, jnp.zeros((128 - hi, TQ), BF16)], axis=0)

    KM = S - NK

    def tie_row(jb, d):
        return ((jb * DH + d) * (KM // 8)) // (NK // 16 * DH)

    def vpu_block(jb, g, sub, qb, pA, ss):
        kw = k_s[g, pl.ds(KM // 2 + 8 * jb, 8), :]
        acc0 = acc1 = None
        for d in range(DH):
            lane = DH * sub + d
            kbw = jnp.broadcast_to(kw[:, lane:lane + 1], (8, 128))
            if d % TS == 0:
                r = tie_row(jb, d)
                cc, r = r // (KC // 8), r % (KC // 8)
                kbw = _paced(kbw, ss[cc][8 * r:8 * r + 8, 128 * (d % 4):128 * (d % 4) + 128])
            kb0 = pltpu.bitcast(kbw << 16, F32)
            kb1 = pltpu.bitcast(kbw & jnp.int32(-65536), F32)
            q = qb[8 * d:8 * d + 8, :]
            t0 = jnp.concatenate([kb0] * (TQ // 128), axis=1) * q
            t1 = jnp.concatenate([kb1] * (TQ // 128), axis=1) * q
            acc0 = t0 if acc0 is None else acc0 + t0
            acc1 = t1 if acc1 is None else acc1 + t1
        e0 = pltpu.bitcast(jnp.exp2(acc0).astype(BF16).astype(F32), I32)
        e1 = pltpu.bitcast(jnp.exp2(acc1).astype(BF16).astype(F32), I32)
        pA[pl.ds(KM // 2 + 8 * jb, 8), :] = jax.lax.shift_right_logical(e0, 16) | e1

    def stages(colA, sub, qb, pA, colB, pB):
        KH = KC // 2
        if colA is not None:
            g = (colA >> 2) & 3
            qm = prep_q(colA, sub, qb)
        if colB is not None:
            h0 = pl.multiple_of((colB & 15) * HP, HP)
            hh = pl.multiple_of((colB & 15) * (HP // 2), HP // 2)
            q0 = pl.multiple_of((colB >> 4) * TQ, TQ)
            acc = jnp.zeros((HP, TQ), F32)
        ss = []
        for c in range(S // KC):
            if colA is not None:
                n = min(KC, KM - c * KC)
                kc = pltpu.bitcast(k_s[g, pl.ds(c * KH, n // 2), :], BF16)
                s = jnp.dot(kc, qm, preferred_element_type=F32)
                pA[pl.ds(c * KH, n // 2), :] = pltpu.bitcast(jnp.exp2(s).astype(BF16), I32)
                ss.append(s)
                for jb in range(NK // 16):
                    if tie_row(jb, DH - 1) // (KC // 8) == c:
                        vpu_block(jb, g, sub, qb, pA, ss)
            if colB is not None:
                p = pltpu.bitcast(pB[pl.ds(c * KH, KH), :], BF16)
                vtc = pltpu.bitcast(vt_s[pl.ds(hh, HP // 2), pl.ds(c * KC, KC)], BF16)
                acc = acc + jnp.dot(vtc, p, preferred_element_type=F32)
        if colB is not None:
            ot_s[pl.ds(h0, HP), pl.ds(q0, TQ)] = acc.astype(BF16)
            l_s[colB & 15, :, pl.ds(q0, TQ)] = acc[DH - 4:DH + 4, :]

    def pair(c, c4, qbs):
        stages(c + 1, (c4 + 1) % 4, qbs[0], p1, c, p0)
        stages(c + 2, (c4 + 2) % 4, qbs[1], p0, c + 1, p1)

    stages(0, 0, qb0, p0, None, None)

    def body(i, carry):
        pair(4 * i, 0, (qb1, qb0))
        pair(4 * i + 2, 2, (qb3, qb2))
        return carry
    jax.lax.fori_loop(0, NCOL // 4 - 1, body, 0)
    pair(NCOL - 4, 0, (qb1, qb0))
    stages(NCOL - 1, 3, qb3, p1, NCOL - 2, p0)
    stages(None, None, None, None, NCOL - 1, p1)

    @pl.when(flag_s[0] == 1)
    def _():
        def col_body(col, carry):
            g = (col >> 2) & 3
            qm = prep_q(col, col & 3)
            h0 = pl.multiple_of((col & 15) * HP, HP)
            hh = pl.multiple_of((col & 15) * (HP // 2), HP // 2)
            q0 = pl.multiple_of((col >> 4) * TQ, TQ)

            def pass1(c, m):
                r0 = pl.multiple_of(c * KC, KC)
                kc = pltpu.bitcast(k_s[g, pl.ds(pl.multiple_of(c * (KC // 2), KC // 2), KC // 2), :], BF16)
                s = jnp.dot(kc, qm, preferred_element_type=F32)
                s0[pl.ds(r0, KC), :] = s
                return jnp.maximum(m, jnp.max(s, axis=0, keepdims=True))
            m = jax.lax.fori_loop(0, S // KC, pass1, jnp.full((1, TQ), -jnp.inf, F32))

            def pass2(c, acc):
                r0 = pl.multiple_of(c * KC, KC)
                p = jnp.exp2(s0[pl.ds(r0, KC), :] - m).astype(BF16)
                vtc = pltpu.bitcast(vt_s[pl.ds(hh, HP // 2), pl.ds(r0, KC)], BF16)
                return acc + jnp.dot(vtc, p, preferred_element_type=F32)
            acc = jax.lax.fori_loop(0, S // KC, pass2, jnp.zeros((HP, TQ), F32))
            ot_s[pl.ds(h0, HP), pl.ds(q0, TQ)] = acc.astype(BF16)
            l_s[col & 15, :, pl.ds(q0, TQ)] = acc[DH - 4:DH + 4, :]
            return carry
        jax.lax.fori_loop(0, NCOL, col_body, 0)

    outs = []
    for r in range(len(OCH)):
        cs = slice(sum(OCH[:r]), sum(OCH[:r + 1]))
        on = jnp.concatenate([ot_s[HP * h:HP * (h + 1), cs].astype(F32) * (1.0 / l_s[h, 4:5, cs]) for h in range(H)], axis=0)
        a = jnp.dot(wot_s[...], on.astype(BF16), preferred_element_type=F32)
        ze = jnp.concatenate([z_s[0, cs, :], z_s[2, cs, :]], axis=1)
        zo = jnp.concatenate([z_s[1, cs, :], z_s[3, cs, :]], axis=1)
        e = jax.lax.dot_general(fi_v[0:DHALF, :], ze, NT, preferred_element_type=F32)
        o = jax.lax.dot_general(fi_v[DHALF:, :], zo, NT, preferred_element_type=F32)
        b = jnp.concatenate([e + o, e - o], axis=0)
        g_ = jax.nn.sigmoid(gate_s[0:1, cs])
        o_v[:, cs] = (b + g_ * (a - b)).astype(BF16)
        cpo = pltpu.make_async_copy(o_v.at[:, cs], out_hbm.at[:, cs], osems.at[r])
        cpo.start()
        outs.append(cpo)
    for cpo in outs:
        cpo.wait()


@jax.jit
def pallas_gated_mix__softmax_full_mha__spectral_gfnet__prompt_kernel(A_x, A_wqkv, A_wo, B_x, B_w_r, B_w_i, gate_w):
    del B_x
    xt = A_x.reshape(S, D).T
    fd, fa, fb, fi = _tables()
    ins = [xt, A_wqkv, A_wo, B_w_r.T, B_w_i.T, gate_w, fd, fa, fb, fi]
    vm = lambda a: pltpu.VMEM(a.shape, a.dtype)
    scratch = [vm(a) for a in ins] + [
        pltpu.VMEM((4, S // 2, 128), I32),
        pltpu.VMEM((D, S), BF16),
        pltpu.VMEM((DP // 2, S), I32),
        pltpu.VMEM((DP, S), BF16),
        pltpu.VMEM((D, DP), BF16),
        pltpu.VMEM((8, S), F32),
        pltpu.VMEM((2 * D + 16, D), BF16),
        pltpu.VMEM((D, D), BF16),
    ] + [pltpu.VMEM((4, S, 128), F32) for _ in range(4)] + [
        pltpu.VMEM((32 * 128, 256), BF16), pltpu.VMEM((4, S, 128), BF16), pltpu.VMEM((2, S, 128), I32),
        pltpu.VMEM((S, TQ), F32), pltpu.VMEM((S // 2, TQ), I32), pltpu.VMEM((S // 2, TQ), I32),
    ] + [pltpu.VMEM((8 * DH, TQ), F32) for _ in range(4)] + [
        pltpu.VMEM((H, 8, S), F32),
        pltpu.VMEM((D, S), BF16), pltpu.SMEM((1,), I32),
        pltpu.SemaphoreType.DMA((len(XCH),)), pltpu.SemaphoreType.DMA((9,)), pltpu.SemaphoreType.DMA((len(OCH),)),
    ]
    out = pl.pallas_call(
        _kernel,
        out_shape=jax.ShapeDtypeStruct((D, S), BF16),
        in_specs=[pl.BlockSpec(memory_space=pltpu.HBM)] * len(ins),
        out_specs=pl.BlockSpec(memory_space=pltpu.HBM),
        scratch_shapes=scratch,
        compiler_params=pltpu.CompilerParams(vmem_limit_bytes=110 * 1024 * 1024, disable_bounds_checks=True,
                                             disable_semaphore_checks=True),
    )(*ins)
    return out.T.reshape(1, S, D)
```
